```python
import jax
import jax.numpy as jnp

def _softmax(x, axis=-1):
    return jax.nn.softmax(x, axis=axis)
def _gelu(x):
    return jax.nn.gelu(x, approximate=True)
def _silu(x):
    return jax.nn.silu(x)
def _sigmoid(x):
    return jax.nn.sigmoid(x)
def _layernorm(x, axis=-1, eps=1e-5):
    m = jnp.mean(x, axis=axis, keepdims=True)
    v = jnp.var(x, axis=axis, keepdims=True)
    return (x - m) / jnp.sqrt(v + eps)
def _scatter_add(tgt, idx, src, axis=0):
    return tgt.at[idx].add(src)
def _segment_sum(src, seg, n):
    return jax.ops.segment_sum(src, seg, n)
class _Rng:
    def __init__(self, key):
        self._k = key
    def _next(self):
        self._k, sub = jax.random.split(self._k)
        return sub
    def normal(self, shape):
        return jax.random.normal(self._next(), shape, dtype=jnp.bfloat16)
    def randint(self, lo, hi, shape):
        return jax.random.randint(self._next(), shape, lo, hi, dtype=jnp.int32)
    def uniform(self, shape, lo=0.0, hi=1.0):
        return jax.random.uniform(self._next(), shape, jnp.bfloat16, lo, hi)
    def permutation(self, n):
        return jax.random.permutation(self._next(), n)


kernel_name = 'sequential_preLN__sliding_local_dilated__glu_gated_geglu__prompt'

def setup_inputs():
    _rng = _Rng(jax.random.key(int.from_bytes(__import__("os").urandom(4), "little")))
    _w = (lambda a: (lambda t: t.astype(jnp.bfloat16) if jnp.issubdtype(t.dtype, jnp.floating) else t)(jnp.asarray(a)))
    def _A_setup():
        B, S, D = 1, 2048, 1024
        return {
            "x": _w((lambda *s: _rng.normal(s) * 0.05)(B, S, D)),
            "wqkv": _w((lambda *s: _rng.normal(s) * 0.05)(D, 3 * D)),
            "wo": _w((lambda *s: _rng.normal(s) * 0.05)(D, D)),
        }
    _A_in = _A_setup()

    def _B_setup():
        B, S, Dm, Df = 1, 2048, 1024, 3584
        return {
            "x": _w((lambda *s: _rng.normal(s) * 0.05)(B, S, Dm)),
            "w_gate": _w((lambda *s: _rng.normal(s) * 0.05)(Dm, Df) * (Dm ** -0.5)),
            "w_up": _w((lambda *s: _rng.normal(s) * 0.05)(Dm, Df) * (Dm ** -0.5)),
            "w_down": _w((lambda *s: _rng.normal(s) * 0.05)(Df, Dm) * (Df ** -0.5)),
        }
    _B_in = _B_setup()

    return {
        "A_x": _A_in["x"],
        "A_wqkv": _A_in["wqkv"],
        "A_wo": _A_in["wo"],
        "B_x": _B_in["x"],
        "B_w_gate": _B_in["w_gate"],
        "B_w_up": _B_in["w_up"],
        "B_w_down": _B_in["w_down"],
    }

def reference(A_x, A_wqkv, A_wo, B_x, B_w_gate, B_w_up, B_w_down):
    def _A_ref(x, wqkv, wo):
        B, S, D = x.shape
        H = 32; Dh = D // H
        W, dil = 8, 2
        qkv = (lambda x, *d: x.transpose(*d))((x @ wqkv).reshape(B, S, 3, H, Dh), 2, 0, 3, 1, 4)
        q, k, v = qkv[0], qkv[1], qkv[2]
        scale = Dh ** -0.5
        pos = jnp.arange(S)
        off = jnp.arange(W) * dil
        idx = pos[:, None] - off[None, :]
        mask = idx >= 0
        idx_c = jnp.where(mask, idx, 0).reshape(-1)
        kg = k[:, :, idx_c, :].reshape(B, H, S, W, Dh)
        vg = v[:, :, idx_c, :].reshape(B, H, S, W, Dh)
        logits = jnp.einsum("bhsd,bhswd->bhsw", q, kg) * scale
        logits = jnp.where(mask[None, None, :, :], logits, -1e9)
        attn = _softmax(logits, axis=-1)
        o = jnp.einsum("bhsw,bhswd->bhsd", attn, vg)
        return (lambda x, *d: x.transpose(*d))(o, 0, 2, 1, 3).reshape(B, S, D) @ wo

    def _B_ref(x, w_gate, w_up, w_down):
        g = jnp.einsum("bsd,df->bsf", x, w_gate)
        u = jnp.einsum("bsd,df->bsf", x, w_up)
        h = _gelu(g) * u
        return jnp.einsum("bsf,fd->bsd", h, w_down)

    x = A_x
    h = x + _A_ref(_layernorm(x, axis=-1), A_wqkv, A_wo)
    h2 = h + _B_ref(_layernorm(h, axis=-1), B_w_gate, B_w_up, B_w_down)
    return h2
```

```python
import functools
import math

import jax
import jax.numpy as jnp
from jax import lax
import jax.experimental.pallas as pl
import jax.experimental.pallas.tpu as pltpu

CFG = dict(T2=256, NH=2, T3=128, FC=512, R=16, PAD=1, FLAGS=None)

S, D, F = 2048, 1024, 3584
H, DH, W, DIL = 32, 32, 8, 2
HALO = 16
NJ = D // 128
T1 = 256
SLAB = 256
NS = D // SLAB
F32, BF16, U32 = jnp.float32, jnp.bfloat16, jnp.uint32


def _ln(x):
    m = jnp.mean(x, axis=-1, keepdims=True)
    c = x - m
    v = jnp.mean(c * c, axis=-1, keepdims=True)
    return c * lax.rsqrt(v + 1e-5)


def _dot(a, b):
    return jnp.dot(a, b, preferred_element_type=F32)


def _geglu(g, u):
    c0 = math.sqrt(2.0 / math.pi)
    z = g * (c0 + (c0 * 0.044715) * (g * g))
    hg = 0.5 * g
    return (hg + hg * jnp.tanh(z)) * u


def _ds(start, size):
    return pl.ds(pl.multiple_of(start, size), size)


def _kernel(x_hbm, wqkv_hbm, wo_hbm, wg_hbm, wu_hbm, wd_hbm, out_hbm,
            xs, xn, wqkv, wo, wg, wu, wd, tmpu, tmpf, q_scr, p_scr, k_scr, v_scr, o_scr, h_scr, hn_scr, a_scr,
            sem_x, sem_w, sem_o, sem_f, sem_out, *, T2, NH, T3, FC, R, PAD):
    N1, N2, N3 = S // T1, S // T2, S // T3
    ST = DH + PAD

    def cp_x(t):
        return pltpu.make_async_copy(x_hbm.at[_ds(t * T1, T1), :], xs.at[_ds(t * T1, T1), :], sem_x.at[t])

    def cp_w(p, s):
        return pltpu.make_async_copy(wqkv_hbm.at[_ds(s * SLAB, SLAB), _ds(p * D, D)],
                                     wqkv.at[p, _ds(s * SLAB, SLAB), :], sem_w.at[p * NS + s])

    def cp_o(j):
        return pltpu.make_async_copy(wo_hbm.at[:, _ds(j * 128, 128)], wo.at[:, _ds(j * 128, 128)], sem_o.at[j])

    cp_ffn = [pltpu.make_async_copy(a, b, sem_f.at[n])
              for n, (a, b) in enumerate(((wg_hbm, wg), (wu_hbm, wu), (wd_hbm, wd)))]

    def cp_out(t):
        return pltpu.make_async_copy(xs.at[_ds(t * T3, T3), :], out_hbm.at[_ds(t * T3, T3), :], sem_out.at[t])

    def spread(ref, val):
        if PAD == 0:
            ref[...] = val
        else:
            for h in range(H):
                ref[h * ST:h * ST + DH, :] = val[h * DH:(h + 1) * DH]

    def permute_cols(p, s):
        rows = _ds(s * SLAB, SLAB)
        spread(tmpu, pltpu.bitcast(wqkv[p, rows, :], U32).T)
        for j in range(NJ):
            t = jnp.concatenate([tmpu[pl.ds(4 * j + e, H, stride=ST), :] for e in range(4)], axis=0)
            wqkv[p, rows, j * 128:(j + 1) * 128] = pltpu.bitcast(t.T, BF16)

    def permute_rows(j):
        cols = _ds(j * 128, 128)
        spread(tmpf, wo[:, cols].astype(F32))
        for d in range(DH):
            wo[d * H:(d + 1) * H, cols] = tmpf[pl.ds(d, H, stride=ST), :].astype(BF16)

    def unit(t):
        return 2 * (t // NS), t % NS

    def ln1(t):
        xn[_ds(t * T1, T1), :] = _ln(xs[_ds(t * T1, T1), :].astype(F32)).astype(BF16)

    cp_x(0).start()
    cp_w(1, 0).start()
    cp_w(1, 1).start()
    k_scr[:, 0:HALO, :] = jnp.zeros((NJ, HALO, 128), F32)
    cp_x(0).wait()
    cp_w(1, 2).start()
    ln1(0)
    cp_w(1, 3).start()

    @pl.loop(0, NS)
    def _(s):
        cp_w(1, s).wait()

        @pl.when(s == 1)
        def _():
            cp_x(1).start()
            cp_w(*unit(0)).start()
            cp_o(0).start()

        @pl.when(s == 3)
        def _():
            cp_x(2).start()
            cp_w(*unit(1)).start()
            cp_o(1).start()
        permute_cols(1, s)

    @pl.loop(0, N1)
    def _(t):
        @pl.when(t + 3 < N1)
        def _():
            cp_x(t + 3).start()

        @pl.when(t + 2 < N1)
        def _():
            cp_w(*unit(t + 2)).start()
            cp_o(t + 2).start()

        @pl.when(t == N1 - 2)
        def _():
            for c in cp_ffn:
                c.start()

        @pl.when(t + 1 < N1)
        def _():
            cp_x(t + 1).wait()
        cp_w(*unit(t)).wait()
        cp_o(t).wait()
        k = _dot(xn[_ds(t * T1, T1), :], wqkv[1])
        for j in range(NJ):
            k_scr[j, pl.ds(pl.multiple_of(HALO + t * T1, HALO), T1), :] = k[:, j * 128:(j + 1) * 128]
        ln1(jnp.minimum(t + 1, N1 - 1))
        permute_cols(*unit(t))
        permute_rows(t)

    TH = T2 // NH
    scale = DH ** -0.5
    v_scr[:, T2:T2 + HALO, :] = jnp.zeros((NJ, HALO, 128), F32)

    @pl.loop(0, N2)
    def _(t):
        base = pl.multiple_of(t * T2, T2)
        v_tail = v_scr[:, T2:T2 + HALO, :]

        def q_proj(a):
            q = _dot(xn[_ds(base + a * TH, TH), :], wqkv[0])
            for j in range(NJ):
                q_scr[j, a * TH:(a + 1) * TH, :] = q[:, j * 128:(j + 1) * 128]

        def v_proj(a):
            v = _dot(xn[_ds(base + a * TH, TH), :], wqkv[2])
            for j in range(NJ):
                vj = v[:, j * 128:(j + 1) * 128]
                v_scr[j, HALO + a * TH:HALO + (a + 1) * TH, :] = vj
                if a == 0:
                    v_scr[j, 0:HALO, :] = jnp.where(t == 0, jnp.broadcast_to(vj[0:1], (HALO, 128)), v_tail[j])

        def probs(a):
            for r0 in range(a * TH, (a + 1) * TH, R):
                qs = [q_scr[j, r0:r0 + R, :] for j in range(NJ)]
                ls = []
                for w in range(W):
                    rows = pl.ds(base + (HALO + r0 - DIL * w), R)
                    acc = qs[0] * k_scr[0, rows, :]
                    for j in range(1, NJ):
                        acc = acc + qs[j] * k_scr[j, rows, :]
                    acc = acc + pltpu.roll(acc, 64, 1)
                    acc = acc + pltpu.roll(acc, 32, 1)
                    acc = acc * scale
                    if r0 < DIL * w:
                        pos = base + r0 + lax.broadcasted_iota(jnp.int32, (R, 128), 0)
                        acc = jnp.where(pos >= DIL * w, acc, -1e9)
                    ls.append(acc)
                m = functools.reduce(jnp.maximum, ls)
                ps = [jnp.exp(l - m) for l in ls]
                inv = 1.0 / functools.reduce(jnp.add, ps)
                for w in range(W):
                    p_scr[w, r0:r0 + R, :] = ps[w] * inv

        def mix(a):
            for r0 in range(a * TH, (a + 1) * TH, R):
                ps = [p_scr[w, r0:r0 + R, :] for w in range(W)]
                for j in range(NJ):
                    acc = ps[0] * v_scr[j, HALO + r0:HALO + r0 + R, :]
                    for w in range(1, W):
                        b = HALO + r0 - DIL * w
                        acc = acc + ps[w] * v_scr[j, b:b + R, :]
                    o_scr[r0:r0 + R, j * 128:(j + 1) * 128] = acc.astype(BF16)

        def o_proj(a):
            rows = _ds(base + a * TH, TH)
            h_scr[rows, :] = xs[rows, :].astype(F32) + _dot(o_scr[a * TH:(a + 1) * TH, :], wo[...])

        for stage in (q_proj, probs, v_proj, mix, o_proj):
            for a in range(NH):
                stage(a)

    def ln2(t, slot):
        hn_scr[slot] = _ln(h_scr[_ds(t * T3, T3), :]).astype(BF16)

    ln2(0, 0)
    for c in cp_ffn:
        c.wait()

    @pl.loop(0, N3)
    def _(t):
        slot = t % 2
        hn = hn_scr[slot]
        for c in range(F // FC):
            g = _dot(hn, wg[:, c * FC:(c + 1) * FC])
            u = _dot(hn, wu[:, c * FC:(c + 1) * FC])
            a_scr[:, c * FC:(c + 1) * FC] = _geglu(g, u).astype(BF16)
        ln2(jnp.minimum(t + 1, N3 - 1), 1 - slot)
        rows = _ds(t * T3, T3)
        xs[rows, :] = (h_scr[rows, :] + _dot(a_scr[...], wd[...])).astype(BF16)
        cp_out(t).start()

    @pl.loop(0, N3)
    def _(t):
        cp_out(t).wait()


@jax.jit
def pallas_sequential_preLN__sliding_local_dilated__glu_gated_geglu__prompt_kernel(
        A_x, A_wqkv, A_wo, B_x, B_w_gate, B_w_up, B_w_down):
    del B_x
    cfg = dict(CFG)
    flags = cfg.pop("FLAGS")
    T2, T3, ST = cfg["T2"], cfg["T3"], DH + cfg["PAD"]
    any_spec = pl.BlockSpec(memory_space=pl.ANY)
    out = pl.pallas_call(
        functools.partial(_kernel, **cfg),
        in_specs=[any_spec] * 6,
        out_specs=any_spec,
        out_shape=jax.ShapeDtypeStruct((S, D), A_x.dtype),
        scratch_shapes=[
            pltpu.VMEM((S, D), BF16), pltpu.VMEM((S, D), BF16),
            pltpu.VMEM((3, D, D), BF16), pltpu.VMEM((D, D), BF16),
            pltpu.VMEM((D, F), BF16), pltpu.VMEM((D, F), BF16), pltpu.VMEM((F, D), BF16),
            pltpu.VMEM((H * ST, 128), U32), pltpu.VMEM((H * ST, 128), F32),
            pltpu.VMEM((NJ, T2, 128), F32), pltpu.VMEM((W, T2, 128), F32),
            pltpu.VMEM((NJ, S + HALO, 128), F32), pltpu.VMEM((NJ, T2 + HALO, 128), F32),
            pltpu.VMEM((T2, D), BF16), pltpu.VMEM((S, D), F32),
            pltpu.VMEM((2, T3, D), BF16), pltpu.VMEM((T3, F), BF16),
            pltpu.SemaphoreType.DMA((S // T1,)), pltpu.SemaphoreType.DMA((3 * NS,)),
            pltpu.SemaphoreType.DMA((NJ,)), pltpu.SemaphoreType.DMA((3,)),
            pltpu.SemaphoreType.DMA((S // T3,)),
        ],
        compiler_params=pltpu.CompilerParams(vmem_limit_bytes=110 * 1024 * 1024, flags=flags),
    )(A_x.reshape(S, D), A_wqkv, A_wo, B_w_gate, B_w_up, B_w_down)
    return out.reshape(A_x.shape)
```

```python
import functools
import math

import jax
import jax.numpy as jnp
from jax import lax
import jax.experimental.pallas as pl
import jax.experimental.pallas.tpu as pltpu

CFG = dict(T2=256, T3=256, FC=512, R=8, RM=16, CH=1, CJ=range(8), CM=((1,3,5,7),(1,3,5,7)), LR=32, LB=1, SHK=1, SHV=1, UP=2, LNP=1, NQ=2, TIE=1, NO=2, SC=0, FLAGS=None)

S, D, F = 2048, 1024, 3584
H, DH, W, DIL = 32, 32, 8, 2
HALO = 16
NJ = D // 128
T1 = 256
SLAB = 256
NS = D // SLAB
ST = DH + 1
F32, BF16, U32 = jnp.float32, jnp.bfloat16, jnp.uint32


def _ln(x):
    m = jnp.mean(x, axis=-1, keepdims=True)
    c = x - m
    v = jnp.mean(c * c, axis=-1, keepdims=True)
    return c * lax.rsqrt(v + 1e-5)


def _dot(a, b):
    return jnp.dot(a, b, preferred_element_type=F32)


def _geglu(g, u):
    c0 = math.sqrt(2.0 / math.pi)
    z = g * (c0 + (c0 * 0.044715) * (g * g))
    hg = 0.5 * g
    return (hg + hg * jnp.tanh(z)) * u


def _ds(start, size):
    if isinstance(start, int):
        return pl.ds(start, size)
    return pl.ds(pl.multiple_of(start, size), size)


def _loop(name, lo, hi):
    def deco(f):
        def g(t):
            if CFG["SC"]:
                with jax.named_scope(name):
                    f(t)
            else:
                f(t)
        pl.loop(lo, hi)(g)
    return deco


def _kernel(x_hbm, wqkv_hbm, wo_hbm, wg_hbm, wu_hbm, wd_hbm, out_hbm,
            xs, xn, wk, wqv, wo, wg, wu, wd, tmpu, tmpf, q_scrs, p_scr, k_scr, v_scrs, tail_scr, o_scr, h_scrs, hn_scr, a_scr,
            sem_x, sem_k, sem_w, sem_o, sem_f, sem_out, *, T2, T3, FC, R, RM, CH, CJ, CM, LR, LB, SHK, SHV, UP, LNP, NQ, TIE, NO, SC):
    N1, N2, N3 = S // T1, S // T2, S // T3

    def cp_x(t):
        return pltpu.make_async_copy(x_hbm.at[_ds(t * T1, T1), :], xs.at[_ds(t * T1, T1), :], sem_x.at[t])

    def cp_k(s):
        return pltpu.make_async_copy(wqkv_hbm.at[_ds(s * SLAB, SLAB), D:2 * D], wk.at[_ds(s * SLAB, SLAB), :], sem_k.at[s])

    def cp_w(u):
        return pltpu.make_async_copy(wqkv_hbm.at[_ds(u % NS * SLAB, SLAB), _ds(u // NS * 2 * D, D)],
                                     wqv.at[_ds(u * SLAB, SLAB), :], sem_w.at[u])

    def cp_o(j):
        return pltpu.make_async_copy(wo_hbm.at[:, _ds(j * 128, 128)], wo.at[:, _ds(j * 128, 128)], sem_o.at[j])

    cp_ffn = [pltpu.make_async_copy(a, b, sem_f.at[n])
              for n, (a, b) in enumerate(((wg_hbm, wg), (wu_hbm, wu), (wd_hbm, wd)))]

    def cp_out(t):
        return pltpu.make_async_copy(xs.at[_ds(t * T3, T3), :], out_hbm.at[_ds(t * T3, T3), :], sem_out.at[t])

    def spread(ref, val):
        for h in range(H):
            ref[h * ST:h * ST + DH, :] = val[h * DH:(h + 1) * DH]

    def permute_cols(ref, s):
        rows = _ds(s * SLAB, SLAB)
        spread(tmpu, pltpu.bitcast(ref[rows, :], U32).T)
        for j in range(NJ):
            t = jnp.concatenate([tmpu[pl.ds(4 * j + e, H, stride=ST), :] for e in range(4)], axis=0)
            ref[rows, j * 128:(j + 1) * 128] = pltpu.bitcast(t.T, BF16)

    def permute_rows(j):
        cols = _ds(j * 128, 128)
        spread(tmpf, wo[:, cols].astype(F32))
        for d in range(DH):
            wo[d * H:(d + 1) * H, cols] = tmpf[pl.ds(d, H, stride=ST), :].astype(BF16)

    def ln1(t):
        xn[_ds(t * T1, T1), :] = _ln(xs[_ds(t * T1, T1), :].astype(F32)).astype(BF16)

    def ln2_chain(a, t, zero):
        TO = T2 // 2
        for r0 in range(0, TO, LR):
            y = _ln(h_scrs[a][_ds(zero + t * TO + TO + r0, LR), :])
            hn_scr[_ds(t * T2 + T2 + a * TO + r0, LR), :] = y.astype(BF16)
            if not isinstance(zero, int):
                tok = functools.reduce(jnp.maximum, [y[i:i + 16, 0:128] for i in range(0, LR, 16)])
                h_scrs[a][0:8, 0:128] = jnp.maximum(tok[0:8], tok[8:16])
        return None if isinstance(zero, int) else tok

    cp_x(0).start()
    for s in range(NS):
        cp_k(s).start()

    def start_step(t):
        if t + 1 < N1:
            cp_x(t + 1).start()
        cp_w(t).start()
        cp_o(t).start()

    if UP == 1:
        for t in range(N1):
            start_step(t)
    k_scr[:, 0:HALO, :] = jnp.zeros((NJ, HALO, 128), F32)
    h_scrs[1][0:T2 // 2, :] = jnp.zeros((T2 // 2, D), F32)
    tail_scr[...] = jnp.zeros((NJ, HALO, 128), F32)
    cp_x(0).wait()
    if UP == 2:
        start_step(0)
    ln1(0)

    @_loop('perm', 0, NS)
    def _(s):
        cp_k(s).wait()
        if UP == 2:
            @pl.when(s == NS - 1)
            def _():
                for t in range(1, N1):
                    start_step(t)
        permute_cols(wk, s)

    @_loop('A1', 0, N1)
    def _(t):
        @pl.when(t == N1 - 2)
        def _():
            for c in cp_ffn:
                c.start()

        @pl.when(t + 1 < N1)
        def _():
            cp_x(t + 1).wait()
        cp_w(t).wait()
        cp_o(t).wait()
        lhs = xn[_ds(t * T1, T1), :]
        if LNP == 0:
            ln1(jnp.minimum(t + 1, N1 - 1))
        k = _dot(lhs, wk[...])
        for j in range(NJ):
            k_scr[j, pl.ds(pl.multiple_of(HALO + t * T1, HALO), T1), :] = k[:, j * 128:(j + 1) * 128]
        if LNP == 1:
            ln1(jnp.minimum(t + 1, N1 - 1))
        permute_cols(wqv, t)
        permute_rows(t)

    @_loop('A2', 0, N2)
    def _(t):
        base = pl.multiple_of(t * T2, T2)

        def windows(ref, j, row, n, mode):
            if mode == 1:
                blk = [ref[j, pl.ds(row - 8 - DIL * w, n + 8), :] for w in range(W // 2)]
                return [b[8:] for b in blk] + [b[:n] for b in blk]
            blk = ref[j, pl.ds(row - HALO, n + HALO), :]
            rot = [blk] + [pltpu.roll(blk, DIL * w, 0) for w in range(1, W // 2)]
            return [b[16:] for b in rot] + [b[8:8 + n] for b in rot]

        TQ = T2 // NQ
        zero = pl.multiple_of(jnp.minimum(t, 0), 32)
        tok = ln2_chain(1, t - 1, zero)
        for a in range(NQ):
            if a == LB:
                xn[_ds(S + zero, 16), 0:128] = tok.astype(BF16)
            q = _dot(xn[_ds(base + a * TQ, TQ), :], wqv[0:D, :])
            for j in range(NJ):
                q_scrs[a][j, 0:TQ, :] = q[:, j * 128:(j + 1) * 128]

        token = [0.0] * NQ
        for r0 in range(0, T2, R):
            a, c0 = divmod(r0, TQ)
            ls = None
            for j in range(NJ):
                qj = q_scrs[a][j, pl.ds(zero + c0, R), :]
                pr = [qj * kw for kw in windows(k_scr, j, base + (HALO + r0), R, SHK)]
                ls = pr if ls is None else [l + p for l, p in zip(ls, pr)]
                if j in CJ:
                    q_scrs[a][0, TQ:TQ + 8, :] = functools.reduce(jnp.maximum, [ls[(j + i * W // CH) % W] for i in range(CH)])[R - 8:]
            for w in range(W):
                acc = ls[w]
                acc = acc + pltpu.roll(acc, 64, 1)
                acc = acc + pltpu.roll(acc, 32, 1)
                if r0 < DIL * w:
                    pos = base + r0 + lax.broadcasted_iota(jnp.int32, (R, 128), 0)
                    acc = jnp.where(pos >= DIL * w, acc, -1e9 * DH ** 0.5)
                ls[w] = acc
            m = functools.reduce(jnp.maximum, ls)
            ps = [jnp.exp2((l - m) * (DH ** -0.5 * math.log2(math.e))) for l in ls]
            inv = 1.0 / functools.reduce(jnp.add, ps)
            for w in range(W):
                p_scr[w, r0:r0 + R, :] = ps[w] * inv

        tails = [tail_scr[j] for j in range(NJ)]
        for a in range(NQ):
            v = _dot(xn[_ds(base + a * TQ, TQ), :], wqv[D:2 * D, :])
            for j in range(NJ):
                vj = v[:, j * 128:(j + 1) * 128]
                if a == 0:
                    tails[j] = jnp.where(t == 0, jnp.broadcast_to(vj[0:1], (HALO, 128)), tails[j])
                v_scrs[a][j, 0:HALO, :] = tails[j]
                v_scrs[a][j, HALO:HALO + TQ, :] = vj
                tails[j] = vj[TQ - HALO:]
        for j in range(NJ):
            tail_scr[j] = tails[j]

        for r0 in range(0, T2, RM):
            a, c0 = divmod(r0, TQ)
            ps = [p_scr[w, r0:r0 + RM, :] for w in range(W)]
            for j in range(NJ):
                vs = windows(v_scrs[a], j, (zero if TIE else 0) + HALO + c0, RM, SHV)
                acc = functools.reduce(jnp.add, [p * vw for p, vw in zip(ps, vs)])
                acc = acc.astype(BF16)
                o_scr[r0:r0 + RM, j * 128:(j + 1) * 128] = acc
                if j in CM[a]:
                    v_scrs[a][0, HALO + TQ:HALO + TQ + 8, :] = pltpu.bitcast(acc, F32)

        TO = T2 // NO
        for a in range(NO):
            rows = _ds(base + a * TO, TO)
            h_scrs[a][_ds(t * TO + TO, TO), :] = xs[rows, :].astype(F32) + _dot(o_scr[a * TO:(a + 1) * TO, :], wo[...])
        ln2_chain(0, t, zero)

    ln2_chain(1, N2 - 1, 0)
    for c in cp_ffn:
        c.wait()

    @_loop('C', 0, N3)
    def _(t):
        hn = hn_scr[_ds(T2 + t * T3, T3), :]
        for c in range(F // FC):
            g = _dot(hn, wg[:, c * FC:(c + 1) * FC])
            u = _dot(hn, wu[:, c * FC:(c + 1) * FC])
            a_scr[:, c * FC:(c + 1) * FC] = _geglu(g, u).astype(BF16)
        y = _dot(a_scr[...], wd[...])
        TO = T2 // 2
        for a in range(2):
            xs[_ds(t * T3 + a * TO, TO), :] = (h_scrs[a][_ds(t * TO + TO, TO), :] + y[a * TO:(a + 1) * TO]).astype(BF16)
        cp_out(t).start()

    @_loop('drain', 0, N3)
    def _(t):
        cp_out(t).wait()


@jax.jit
def pallas_sequential_preLN__sliding_local_dilated__glu_gated_geglu__prompt_kernel(
        A_x, A_wqkv, A_wo, B_x, B_w_gate, B_w_up, B_w_down):
    del B_x
    cfg = dict(CFG)
    flags = cfg.pop("FLAGS")
    T2, T3, NQ = cfg["T2"], cfg["T3"], cfg["NQ"]
    TQ = T2 // NQ
    any_spec = pl.BlockSpec(memory_space=pl.ANY)
    out = pl.pallas_call(
        functools.partial(_kernel, **cfg),
        in_specs=[any_spec] * 6,
        out_specs=any_spec,
        out_shape=jax.ShapeDtypeStruct((S, D), A_x.dtype),
        scratch_shapes=[
            pltpu.VMEM((S, D), BF16), pltpu.VMEM((S + 16, D), BF16),
            pltpu.VMEM((D, D), BF16), pltpu.VMEM((2 * D, D), BF16), pltpu.VMEM((D, D), BF16),
            pltpu.VMEM((D, F), BF16), pltpu.VMEM((D, F), BF16), pltpu.VMEM((F, D), BF16),
            pltpu.VMEM((H * ST, 128), U32), pltpu.VMEM((H * ST, 128), F32),
            [pltpu.VMEM((NJ, TQ + 8, 128), F32)] * NQ, pltpu.VMEM((W, T2, 128), F32), pltpu.VMEM((NJ, HALO + S, 128), F32),
            [pltpu.VMEM((NJ, HALO + TQ + 8, 128), F32)] * NQ, pltpu.VMEM((NJ, HALO, 128), F32), pltpu.VMEM((T2, D), BF16), [pltpu.VMEM((S // 2 + T2 // 2, D), F32)] * 2,
            pltpu.VMEM((T2 + S, D), BF16), pltpu.VMEM((T3, F), BF16),
            pltpu.SemaphoreType.DMA((S // T1,)), pltpu.SemaphoreType.DMA((NS,)), pltpu.SemaphoreType.DMA((2 * NS,)),
            pltpu.SemaphoreType.DMA((NJ,)), pltpu.SemaphoreType.DMA((3,)),
            pltpu.SemaphoreType.DMA((S // T3,)),
        ],
        compiler_params=pltpu.CompilerParams(vmem_limit_bytes=110 * 1024 * 1024, flags=flags),
    )(A_x.reshape(S, D), A_wqkv, A_wo, B_w_gate, B_w_up, B_w_down)
    return out.reshape(A_x.shape)
```

```python
import functools
import math

import jax
import jax.numpy as jnp
from jax import lax
import jax.experimental.pallas as pl
import jax.experimental.pallas.tpu as pltpu

CFG = dict(T2=256, T3=256, FC=128, DC=128, ORD=(1,3,6,4,0,2,5), R=8, RM=16, CH=1, CJ=range(8), CM=((1,3,5,7),(1,3,5,7)), LR=32, LB=1, SHK=1, SHV=1, UP=((0,),(1,),(2,),(3,)), LATE=2, OE=1, L1=64, NQ=2, TIE=1, NO=2, SC=0, FLAGS=None)

S, D, F = 2048, 1024, 3584
H, DH, W, DIL = 32, 32, 8, 2
HALO = 16
NJ = D // 128
T1 = 256
SLAB = 256
NS = D // SLAB
ST = DH + 1
F32, BF16, U32 = jnp.float32, jnp.bfloat16, jnp.uint32


def _ln(x):
    m = jnp.mean(x, axis=-1, keepdims=True)
    c = x - m
    v = jnp.mean(c * c, axis=-1, keepdims=True)
    return c * lax.rsqrt(v + 1e-5)


def _dot(a, b):
    return jnp.dot(a, b, preferred_element_type=F32)


def _geglu(g, u):
    c0 = math.sqrt(2.0 / math.pi)
    z = g * (c0 + (c0 * 0.044715) * (g * g))
    hg = 0.5 * g
    return (hg + hg * jnp.tanh(z)) * u


def _ds(start, size):
    if isinstance(start, int):
        return pl.ds(start, size)
    return pl.ds(pl.multiple_of(start, size & -size), size)


def _loop(name, lo, hi):
    def deco(f):
        def g(t):
            if CFG["SC"]:
                with jax.named_scope(name):
                    f(t)
            else:
                f(t)
        pl.loop(lo, hi)(g)
    return deco


def _pack(x):
    return pltpu.bitcast(x.astype(BF16), U32)


def _unpack(x):
    return pltpu.bitcast(x, BF16)


def _lhs_terms(a11, a12, a21, a22):
    return [_pack(t) for t in (a11 + a22, a21 + a22, a11, a22, a11 + a12, a21 - a11, a12 - a22)]


def _combine(m):
    return m[3] + m[6] - m[4] + m[0], m[4] + m[2], m[1] + m[3], m[0] - m[1] + m[2] + m[5]


def _kernel(x_hbm, wqkv_hbm, wo_hbm, wg_hbm, wu_hbm, wd_hbm, out_hbm,
            xs, xn, wk, wqv, wo, wg, wu, wd, tmpu, tmpf, q_scrs, p_scr, k_scr, v_scrs, tail_scr, o_scr, h_scrs, hn_scr, a_scr,
            sem_x, sem_k, sem_w, sem_o, sem_f, sem_out, *, T2, T3, FC, DC, ORD, R, RM, CH, CJ, CM, LR, LB, SHK, SHV, UP, LATE, OE, L1, NQ, TIE, NO, SC):
    N1, N2, N3 = S // T1, S // T2, S // T3

    def cp_x(t):
        return pltpu.make_async_copy(x_hbm.at[_ds(t * T1, T1), :], xs.at[_ds(t * T1, T1), :], sem_x.at[t])

    def cp_k(s):
        return pltpu.make_async_copy(wqkv_hbm.at[_ds(s * SLAB, SLAB), D:2 * D], wk.at[_ds(s * SLAB, SLAB), :], sem_k.at[s])

    def cp_w(u):
        return pltpu.make_async_copy(wqkv_hbm.at[_ds(u % NS * SLAB, SLAB), _ds(u // NS * 2 * D, D)],
                                     wqv.at[_ds(u * SLAB, SLAB), :], sem_w.at[u])

    def cp_o(j):
        return pltpu.make_async_copy(wo_hbm.at[:, _ds(j * 128, 128)], wo.at[:, _ds(j * 128, 128)], sem_o.at[j])

    cp_ffn = [pltpu.make_async_copy(a, b, sem_f.at[n])
              for n, (a, b) in enumerate(((wg_hbm, wg), (wu_hbm, wu), (wd_hbm, wd)))]

    def cp_out(t):
        return pltpu.make_async_copy(xs.at[_ds(t * T3, T3), :], out_hbm.at[_ds(t * T3, T3), :], sem_out.at[t])

    def spread(ref, val):
        for h in range(H):
            ref[h * ST:h * ST + DH, :] = val[h * DH:(h + 1) * DH]

    def permute_cols(ref, s):
        rows = _ds(s * SLAB, SLAB)
        spread(tmpu, pltpu.bitcast(ref[rows, :], U32).T)
        for j in range(NJ):
            t = jnp.concatenate([tmpu[pl.ds(4 * j + e, H, stride=ST), :] for e in range(4)], axis=0)
            ref[rows, j * 128:(j + 1) * 128] = pltpu.bitcast(t.T, BF16)

    def permute_rows(j):
        cols = _ds(j * 128, 128)
        spread(tmpf, wo[:, cols].astype(F32))
        for d in range(DH):
            wo[d * H:(d + 1) * H, cols] = tmpf[pl.ds(d, H, stride=ST), :].astype(BF16)

    def ln1(t, zero):
        n = T1 if isinstance(zero, int) else L1
        for r0 in range(0, T1, n):
            y = _ln(xs[_ds(zero + t * T1 + r0, n), :].astype(F32)).astype(BF16)
            xn[_ds(t * T1 + r0, n), :] = y
            if n < T1:
                xs[S:S + 16, 0:128] = functools.reduce(jnp.maximum, [y[i:i + 16, 0:128] for i in range(0, n, 16)])

    def ln2_chain(a, t, zero):
        TO = T2 // 2
        for r0 in range(0, TO, LR):
            y = _ln(h_scrs[a][_ds(zero + t * TO + TO + r0, LR), :])
            n = LR // 2
            for i, term in enumerate(_lhs_terms(y[:n, :D // 2], y[:n, D // 2:], y[n:, :D // 2], y[n:, D // 2:])):
                hn_scr[i, _ds((t * T2 + T2 + a * TO + r0) // 4, n // 2), :] = term
            if not isinstance(zero, int):
                tok = functools.reduce(jnp.maximum, [y[i:i + 16, 0:128] for i in range(0, LR, 16)])
                h_scrs[a][0:8, 0:128] = jnp.maximum(tok[0:8], tok[8:16])
        return None if isinstance(zero, int) else tok

    def start_step(t):
        if t + 1 < N1:
            cp_x(t + 1).start()
        cp_w(t).start()
        if t >= OE:
            cp_o(t).start()

    cp_k(0).start()
    cp_k(1).start()
    for t in range(OE):
        cp_o(t).start()
    k_scr[:, 0:HALO, :] = jnp.zeros((NJ, HALO, 128), F32)
    h_scrs[1][0:T2 // 2, :] = jnp.zeros((T2 // 2, D), F32)
    tail_scr[...] = jnp.zeros((NJ, HALO, 128), F32)

    @_loop('perm', 0, NS)
    def _(s):
        cp_k(s).wait()
        for i, nxt in enumerate(UP):
            @pl.when(s == i)
            def _():
                for n in nxt:
                    if n < 2:
                        cp_k(n + 2).start()
                    elif n == 2:
                        cp_x(0).start()
                    else:
                        start_step(n - 3)
        permute_cols(wk, s)

    cp_x(0).wait()
    ln1(0, 0)
    for t in range(1, LATE):
        start_step(t)

    @_loop('A1', 0, N1)
    def _(t):
        @pl.when(t + 1 < N1)
        def _():
            cp_x(t + 1).wait()
        cp_w(t).wait()
        cp_o(t).wait()

        @pl.when(t + LATE + 1 < N1)
        def _():
            cp_x(t + LATE + 1).start()

        @pl.when(t + LATE < N1)
        def _():
            cp_w(t + LATE).start()
            cp_o(t + LATE).start()

        @pl.when(t == N1 - LATE)
        def _():
            for c in cp_ffn:
                c.start()
        lhs = xn[_ds(t * T1, T1), :]
        k = _dot(lhs, wk[...])
        for j in range(NJ):
            k_scr[j, pl.ds(pl.multiple_of(HALO + t * T1, HALO), T1), :] = k[:, j * 128:(j + 1) * 128]
        ln1(jnp.minimum(t + 1, N1 - 1), pl.multiple_of(jnp.minimum(t, 0), T1))
        permute_cols(wqv, t)
        permute_rows(t)

    @_loop('A2', 0, N2)
    def _(t):
        base = pl.multiple_of(t * T2, T2)

        def windows(ref, j, row, n, mode):
            if mode == 1:
                blk = [ref[j, pl.ds(row - 8 - DIL * w, n + 8), :] for w in range(W // 2)]
                return [b[8:] for b in blk] + [b[:n] for b in blk]
            blk = ref[j, pl.ds(row - HALO, n + HALO), :]
            rot = [blk] + [pltpu.roll(blk, DIL * w, 0) for w in range(1, W // 2)]
            return [b[16:] for b in rot] + [b[8:8 + n] for b in rot]

        TQ = T2 // NQ
        zero = pl.multiple_of(jnp.minimum(t, 0), 32)
        tok = ln2_chain(1, t - 1, zero)
        for a in range(NQ):
            if a == LB:
                xn[_ds(S + zero, 16), 0:128] = tok.astype(BF16)
            q = _dot(xn[_ds(base + a * TQ, TQ), :], wqv[0:D, :])
            for j in range(NJ):
                q_scrs[a][j, 0:TQ, :] = q[:, j * 128:(j + 1) * 128]

        token = [0.0] * NQ
        for r0 in range(0, T2, R):
            a, c0 = divmod(r0, TQ)
            ls = None
            for j in range(NJ):
                qj = q_scrs[a][j, pl.ds(zero + c0, R), :]
                pr = [qj * kw for kw in windows(k_scr, j, base + (HALO + r0), R, SHK)]
                ls = pr if ls is None else [l + p for l, p in zip(ls, pr)]
                if j in CJ:
                    q_scrs[a][0, TQ:TQ + 8, :] = functools.reduce(jnp.maximum, [ls[(j + i * W // CH) % W] for i in range(CH)])[R - 8:]
            for w in range(W):
                acc = ls[w]
                acc = acc + pltpu.roll(acc, 64, 1)
                acc = acc + pltpu.roll(acc, 32, 1)
                if r0 < DIL * w:
                    pos = base + r0 + lax.broadcasted_iota(jnp.int32, (R, 128), 0)
                    acc = jnp.where(pos >= DIL * w, acc, -1e9 * DH ** 0.5)
                ls[w] = acc
            m = functools.reduce(jnp.maximum, ls)
            ps = [jnp.exp2((l - m) * (DH ** -0.5 * math.log2(math.e))) for l in ls]
            inv = 1.0 / functools.reduce(jnp.add, ps)
            for w in range(W):
                p_scr[w, r0:r0 + R, :] = ps[w] * inv

        tails = [tail_scr[j] for j in range(NJ)]
        for a in range(NQ):
            v = _dot(xn[_ds(base + a * TQ, TQ), :], wqv[D:2 * D, :])
            for j in range(NJ):
                vj = v[:, j * 128:(j + 1) * 128]
                if a == 0:
                    tails[j] = jnp.where(t == 0, jnp.broadcast_to(vj[0:1], (HALO, 128)), tails[j])
                v_scrs[a][j, 0:HALO, :] = tails[j]
                v_scrs[a][j, HALO:HALO + TQ, :] = vj
                tails[j] = vj[TQ - HALO:]
        for j in range(NJ):
            tail_scr[j] = tails[j]

        for r0 in range(0, T2, RM):
            a, c0 = divmod(r0, TQ)
            ps = [p_scr[w, r0:r0 + RM, :] for w in range(W)]
            for j in range(NJ):
                vs = windows(v_scrs[a], j, (zero if TIE else 0) + HALO + c0, RM, SHV)
                acc = functools.reduce(jnp.add, [p * vw for p, vw in zip(ps, vs)])
                acc = acc.astype(BF16)
                o_scr[r0:r0 + RM, j * 128:(j + 1) * 128] = acc
                if j in CM[a]:
                    v_scrs[a][0, HALO + TQ:HALO + TQ + 8, :] = pltpu.bitcast(acc, F32)

        TO = T2 // NO
        for a in range(NO):
            rows = _ds(base + a * TO, TO)
            h_scrs[a][_ds(t * TO + TO, TO), :] = xs[rows, :].astype(F32) + _dot(o_scr[a * TO:(a + 1) * TO, :], wo[...])
        ln2_chain(0, t, zero)

    ln2_chain(1, N2 - 1, 0)
    for c in cp_ffn:
        c.wait()

    def strassen(lhs, w, c, m):
        k2, n2 = w.shape[0] // 2, w.shape[1] // 2
        b11, b12, b21, b22 = (w[r:r + k2, j + c:j + c + m] for r in (0, k2) for j in (0, n2))
        add = lambda x, y: (x.astype(F32) + y.astype(F32)).astype(BF16)
        sub = lambda x, y: (x.astype(F32) - y.astype(F32)).astype(BF16)
        rhs = (add(b11, b22), b11, sub(b12, b22), sub(b21, b11), b22, add(b11, b12), add(b21, b22))
        prod = {i: _dot(_unpack(lhs(i)), rhs[i]) for i in ORD}
        return _combine(prod)

    @_loop('C', 0, N3)
    def _(t):
        hn = lambda i: hn_scr[i, _ds((T2 + t * T3) // 4, T3 // 4), :]
        for c in range(0, F // 2, FC):
            g = strassen(hn, wg, c, FC)
            u = strassen(hn, wu, c, FC)
            for i, term in enumerate(_lhs_terms(*map(_geglu, g, u))):
                a_scr[i, :, c:c + FC] = term
        TO, n = T2 // 2, LR // 2
        for c in range(0, D // 2, DC):
            y = strassen(lambda i: a_scr[i], wd, c, DC)
            for q in range(4):
                cols = slice(q % 2 * D // 2 + c, q % 2 * D // 2 + c + DC)
                for i in range(T3 // LR):
                    a, r = divmod(i * LR + q // 2 * n, TO)
                    xs[_ds(t * T3 + a * TO + r, n), cols] = (
                        h_scrs[a][_ds(t * TO + TO + r, n), cols] + y[q][i * n:(i + 1) * n]).astype(BF16)
        cp_out(t).start()

    @_loop('drain', 0, N3)
    def _(t):
        cp_out(t).wait()


@jax.jit
def pallas_sequential_preLN__sliding_local_dilated__glu_gated_geglu__prompt_kernel(
        A_x, A_wqkv, A_wo, B_x, B_w_gate, B_w_up, B_w_down):
    del B_x
    cfg = dict(CFG)
    flags = cfg.pop("FLAGS")
    T2, T3, NQ = cfg["T2"], cfg["T3"], cfg["NQ"]
    TQ = T2 // NQ
    any_spec = pl.BlockSpec(memory_space=pl.ANY)
    out = pl.pallas_call(
        functools.partial(_kernel, **cfg),
        in_specs=[any_spec] * 6,
        out_specs=any_spec,
        out_shape=jax.ShapeDtypeStruct((S, D), A_x.dtype),
        scratch_shapes=[
            pltpu.VMEM((S + 16, D), BF16), pltpu.VMEM((S + 16, D), BF16),
            pltpu.VMEM((D, D), BF16), pltpu.VMEM((2 * D, D), BF16), pltpu.VMEM((D, D), BF16),
            pltpu.VMEM((D, F), BF16), pltpu.VMEM((D, F), BF16), pltpu.VMEM((F, D), BF16),
            pltpu.VMEM((H * ST, 128), U32), pltpu.VMEM((H * ST, 128), F32),
            [pltpu.VMEM((NJ, TQ + 8, 128), F32)] * NQ, pltpu.VMEM((W, T2, 128), F32), pltpu.VMEM((NJ, HALO + S, 128), F32),
            [pltpu.VMEM((NJ, HALO + TQ + 8, 128), F32)] * NQ, pltpu.VMEM((NJ, HALO, 128), F32), pltpu.VMEM((T2, D), BF16), [pltpu.VMEM((S // 2 + T2 // 2, D), F32)] * 2,
            pltpu.VMEM((7, (T2 + S) // 4, D // 2), U32), pltpu.VMEM((7, T3 // 4, F // 2), U32),
            pltpu.SemaphoreType.DMA((S // T1,)), pltpu.SemaphoreType.DMA((NS,)), pltpu.SemaphoreType.DMA((2 * NS,)),
            pltpu.SemaphoreType.DMA((NJ,)), pltpu.SemaphoreType.DMA((3,)),
            pltpu.SemaphoreType.DMA((S // T3,)),
        ],
        compiler_params=pltpu.CompilerParams(vmem_limit_bytes=110 * 1024 * 1024, flags=flags),
    )(A_x.reshape(S, D), A_wqkv, A_wo, B_w_gate, B_w_up, B_w_down)
    return out.reshape(A_x.shape)
```

```python
import functools
import math

import jax
import jax.numpy as jnp
from jax import lax
import jax.experimental.pallas as pl
import jax.experimental.pallas.tpu as pltpu

CFG = dict(CJ=range(8), RQ=8, CH=2, PR=1, CM=range(8), CJW=range(8), CMW=range(8), L1=2, EX=0, L2=2, NW=128, SC=0, FLAGS=None)

S, D, F = 2048, 1024, 3584
H, DH, W, DIL = 32, 32, 8, 2
T = 256
NT = S // T
NS = D // T
NJ = D // 128
HALO = 16
P0 = T + HALO
ST = DH + 1
G = 32
ORDER = (1, 3, 6, 4, 0, 2, 5)
F32, BF16, U32 = jnp.float32, jnp.bfloat16, jnp.uint32


def _ln(x):
    m = jnp.mean(x, axis=-1, keepdims=True)
    c = x - m
    v = jnp.mean(c * c, axis=-1, keepdims=True)
    return c * lax.rsqrt(v + 1e-5)


def _geglu(g, u):
    c0 = math.sqrt(2.0 / math.pi)
    z = g * (c0 + (c0 * 0.044715) * (g * g))
    hg = 0.5 * g
    return (hg + hg * jnp.tanh(z)) * u


def _ds(start, size, align=None):
    if isinstance(start, int):
        return pl.ds(start, size)
    return pl.ds(pl.multiple_of(start, align or size), size)


def _tile(j):
    return slice(j * 128, (j + 1) * 128)


def _pack(x):
    return pltpu.bitcast(x.astype(BF16), U32)


def _unpack(x):
    return pltpu.bitcast(x, BF16)


def _lhs_terms(a11, a12, a21, a22):
    return a11 + a22, a21 + a22, a11, a22, a11 + a12, a21 - a11, a12 - a22


def _rhs_terms(b11, b12, b21, b22):
    f11, f12, f21, f22 = (b.astype(F32) for b in (b11, b12, b21, b22))
    return f11 + f22, b11, f12 - f22, f21 - f11, b22, f11 + f12, f21 + f22


def _strassen(lhs, rhs):
    m = {i: jnp.dot(lhs(i), rhs(i), preferred_element_type=F32) for i in ORDER}
    return m[3] + m[6] - m[4] + m[0], m[4] + m[2], m[1] + m[3], m[0] - m[1] + m[2] + m[5]


def _row_groups(c):
    n = G // 2
    return [(i * G + q // 2 * n, q % 2, c[q][i * n:(i + 1) * n]) for q in range(4) for i in range(T // G)]


def _even_odd(y):
    return [jnp.concatenate([y[:, _tile(j)] for j in range(e, NJ, 2)], axis=1) for e in range(2)]


def _loop(name, n):
    def deco(f):
        def g(t):
            if CFG["SC"]:
                with jax.named_scope(name):
                    f(t)
            else:
                f(t)
        pl.loop(0, n)(g)
    return deco


def _kernel(x_hbm, wqkv_hbm, wo_hbm, wg_hbm, wu_hbm, wd_hbm, out_hbm,
            xs, raw, raw_o, wk, wqv, wo, wg, wu, wd, tmp_c, tmp_r, xn, qv, ks, ps, os, hs, hn, act,
            sem_x, sem_w, sem_o, sem_f, sem_out, *, CJ, RQ, CH, PR, CM, CJW, CMW, L1, EX, L2, NW, SC):
    def cp_x(t):
        return pltpu.make_async_copy(x_hbm.at[_ds(t * T, T), :], xs.at[_ds(t * T, T), :], sem_x.at[t])

    def cp_w(u):
        col = jnp.where(u < NS, 1, u // NS * 2 - 2) if not isinstance(u, int) else (1, 0, 2)[u // NS]
        return pltpu.make_async_copy(wqkv_hbm.at[_ds(u % NS * T, T), _ds(col * D, D)],
                                     raw.at[_ds(u * T, T), :], sem_w.at[u])

    def cp_o(j):
        return pltpu.make_async_copy(wo_hbm.at[:, _ds(j * 128, 128)], raw_o.at[:, _ds(j * 128, 128)], sem_o.at[j])

    cp_ffn = [pltpu.make_async_copy(src, dst, sem_f.at[i])
              for i, (src, dst) in enumerate(((wg_hbm, wg), (wu_hbm, wu), (wd_hbm, wd)))]

    def cp_out(t):
        return pltpu.make_async_copy(xs.at[_ds(t * T, T), :], out_hbm.at[_ds(t * T, T), :], sem_out.at[t])

    def prepare_cols(u, dst, s):
        cols = pltpu.bitcast(raw[_ds(u * T, T), :], U32).T
        for h in range(H):
            tmp_c[h * ST:h * ST + DH, :] = cols[h * DH:(h + 1) * DH]

        def tile(j):
            rows = [tmp_c[pl.ds(4 * j + e, H, stride=ST), :] for e in range(4)]
            return _unpack(jnp.concatenate(rows, axis=0).T)

        for j in range(NJ // 2):
            left, right = tile(j), tile(j + NJ // 2)
            for i, term in enumerate(_rhs_terms(left[:128], right[:128], left[128:], right[128:])):
                dst[i, _ds(s * 64, 64), _tile(j)] = _pack(term)
            yield _pack(term)[-8:]

    def prepare_rows(j, half):
        for e in range(2):
            for h in range(H):
                rows = raw_o[_ds(h * DH + half * (DH // 2), DH // 2), _ds((j + e * NJ // 2) * 128, 128)]
                tmp_r[e, h * 9:h * 9 + 8, :] = pltpu.bitcast(rows, U32)
        for d in (0, 1, 2, 3, 8, 9, 10, 11):
            words = [tmp_r[e, pl.ds((d + k) // 2, H, stride=9), :] for k in (0, 4) for e in range(2)]
            quads = [pltpu.bitcast(w >> 16 << 16 if d % 2 else w << 16, F32) for w in words]
            for i, term in enumerate(_rhs_terms(*quads)):
                wo[i, _ds(half * 128 + (d // 8 * 4 + d % 8) * 16, 16), _ds(j * 128, 128)] = _pack(term)
            if d % 2:
                yield _pack(term)[-8:]

    def norm(src, base, off, split, dst, drow, never=None, link=1, extra=(), n=T):
        tok, toks = None, []
        for g in range(n // G):
            x = src[_ds(base + (off + g * G), G), :].astype(F32)
            if tok is not None:
                first = jnp.where(never, jnp.concatenate([tok] * (G // 8), axis=0), x[:, :128])
                x = jnp.concatenate([first, x[:, 128:]], axis=1)
            y = _ln(x)
            terms = [_pack(a) for a in _lhs_terms(*split(y[:G // 2]), *split(y[G // 2:]))]
            for i, term in enumerate(terms):
                dst[i, _ds(drow + g * G // 4, G // 4), :] = term
            toks.append(terms[0][:, :128])
            if never is not None and (g + 1) % link == 0:
                toks += [e[g // link] for e in extra if g // link < len(e)]
                tok, toks = pltpu.bitcast(functools.reduce(jnp.bitwise_or, toks), F32), []

    def halves(y):
        return y[:, :D // 2], y[:, D // 2:]

    def windows(ref, j, base, row, n):
        blk = [ref[j, pl.ds(base + (row - 8 - DIL * w), n + 8), :] for w in range(W // 2)]
        return [b[8:] for b in blk] + [b[:n] for b in blk]

    def attend(base, off, n, zero, maybe_first, links_qk, links_pv):
        def fold(vals):
            return functools.reduce(jnp.maximum, [v[i:i + 8] for v in vals for i in range(0, v.shape[0], 8)])

        def logits(r):
            ls = None
            for j in range(NJ):
                q = qv[j, _ds(base + (P0 + off + r), RQ), :]
                pr = [q * k for k in windows(ks, j, zero + base, P0 + off + r, RQ)]
                ls = pr if ls is None else [l + p for l, p in zip(ls, pr)]
                if j in links_qk:
                    ks[0, 0:8, :] = fold([ls[(j + i * W // CH) % W] for i in range(CH)])
            return ls

        def softmax(r, ls):
            ls = [l + pltpu.roll(l, 64, 1) for l in ls]
            ls = [l + pltpu.roll(l, 32, 1) for l in ls]
            if maybe_first and r < HALO:
                pos = base + (off + r) + lax.broadcasted_iota(jnp.int32, (RQ, 128), 0)
                ls = [jnp.where(pos >= DIL * w, l, -1e9 * DH ** 0.5) for w, l in enumerate(ls)]
            m = functools.reduce(jnp.maximum, ls)
            es = [jnp.exp2((l - m) * (DH ** -0.5 * math.log2(math.e))) for l in ls]
            inv = 1.0 / functools.reduce(jnp.add, es)
            for w in range(W):
                ps[w, r:r + RQ, :] = es[w] * inv

        def mix(r):
            p = None
            for j in range(NJ):
                p = [ps[w, _ds(zero + r, 16), :] if p is None or (j - 1 in links_pv and w < PR) else p[w] for w in range(W)]
                acc = functools.reduce(jnp.add, [a * v for a, v in zip(p, windows(qv, NJ + j, base, P0 + off + r, 16))])
                os[_ds(base + (T + off + r), 16), _tile(j)] = acc
                if j in links_pv:
                    tok = fold([acc])
                    ps[0, T:T + 8, :] = tok
            return tok

        pending = []
        for r in range(0, n + 32, 16):
            new = [(r + i, logits(r + i)) for i in range(0, 16, RQ)] if r < n else []
            if new:
                ps[0, T:T + 8, :] = new[-1][1][NJ - 1][-8:]
            if r >= 32:
                ks[0, 0:8, :] = mix(r - 32)
            for job in pending:
                softmax(*job)
            pending = new

    def start_step(t):
        cp_x(t + 1).start()
        cp_w(NS + t).start()

    cp_w(0).start()
    cp_w(1).start()
    cp_o(0).start()
    cp_o(NJ // 2).start()
    for ref in (qv, ks):
        ref[:, 0:P0, :] = jnp.zeros((ref.shape[0], P0, 128), F32)
    hs[T:T + T // 4, :] = jnp.zeros((T // 4, D), F32)

    @_loop('perm', NS)
    def _(s):
        cp_w(s).wait()
        for i, start in enumerate((cp_w(2).start, cp_w(3).start, cp_x(0).start, lambda: start_step(0))):
            pl.when(s == i)(start)
        list(prepare_cols(s, wk, s))

    cp_x(0).wait()
    norm(xs, 0, 0, _even_odd, xn, 0)
    start_step(1)

    def project(t, base, w, k0, out, plane):
        lhs = [_unpack(xn[i, _ds(t * (T // 4), T // 4), :]) for i in range(7)]
        for c in range(0, D // 2, NW):
            res = _strassen(lambda i: lhs[i], lambda i: _unpack(w[i, k0:k0 + D // 4, c:c + NW]))
            for r, half, val in _row_groups(res):
                for j in range(NW // 128):
                    out[plane + half * NJ // 2 + c // 128 + j, _ds(base + (P0 + r), G // 2), :] = val[:, _tile(j)]

    @_loop('K', NT)
    def _(t):
        pl.when(t + 1 < NT)(lambda: cp_x(t + 1).wait())
        cp_w(NS + t).wait()

        @pl.when(t % 2 == 0)
        def _():
            cp_o(t // 2).wait()
            cp_o(t // 2 + NJ // 2).wait()

            @pl.when(t + 2 < NT)
            def _():
                cp_o(t // 2 + 1).start()
                cp_o(t // 2 + 1 + NJ // 2).start()

        pl.when(t + 3 < NT)(lambda: cp_x(t + 3).start())
        pl.when(t + 2 < NT)(lambda: cp_w(NS + t + 2).start())

        @pl.when(t == NT - 2)
        def _():
            for c in cp_ffn:
                c.start()

        project(t, t * T, wk, 0, ks, 0)
        nxt = jnp.minimum(t + 1, NT - 1)
        extra = [list(prepare_cols(NS + t, wqv, t)), list(prepare_rows(t // 2, t % 2))]
        norm(xs, nxt * T, 0, _even_odd, xn, nxt * (T // 4), t < 0, L1, extra[EX:])

    @_loop('QV', NT)
    def _(t):
        @pl.when(t == 1)
        def _():
            for j in range(NJ, 2 * NJ):
                qv[j, T:P0, :] = jnp.broadcast_to(qv[j, P0:P0 + 1, :], (HALO, 128))

        base = pl.multiple_of(t * T, T)
        attend(base, -T, T, pl.multiple_of(jnp.minimum(t, 0), T), True, CJ, CM)
        project(t, base, wqv, 0, qv, 0)
        project(t, base, wqv, D // 4, qv, NJ)

    @_loop('O', NT)
    def _(t):
        zero = jnp.minimum(t, 0)
        base = pl.multiple_of(t * T, T)
        part = jnp.clip(t - 1, 0, 3) * (T // 4)
        norm(hs, part, T, halves, hn, (T + part) // 4, n=T // 4)
        blocks = [jnp.concatenate([os[_ds(T + t * T + g * G + e * G // 2, G // 2), :] for g in range(T // G)], axis=0)
                  for e in range(2)]
        lhs = [a.astype(BF16) for a in _lhs_terms(*_even_odd(blocks[0]), *_even_odd(blocks[1]))]
        attend(jnp.minimum(t * 48, T - 48), S - T, 48, zero, False, CJW, CMW)
        for c in range(0, D // 2, NW):
            res = _strassen(lambda i: lhs[i], lambda i: _unpack(wo[i, :, c:c + NW]))
            for r, half, val in _row_groups(res):
                cols = pl.ds(half * D // 2 + c, NW)
                hs[_ds(base + (T + r), G // 2), cols] = xs[_ds(base + r, G // 2), cols].astype(F32) + val

    for c in cp_ffn:
        c.wait()

    @_loop('FFN', NT)
    def _(t):
        def matmul(lhs, w, c):
            k2, n2 = w.shape[0] // 2, w.shape[1] // 2
            rhs = _rhs_terms(*(w[r:r + k2, j + c:j + c + 128] for r in (0, k2) for j in (0, n2)))
            return _strassen(lhs, lambda i: rhs[i].astype(BF16))

        lhs = [_unpack(hn[i, _ds((t + 1) * (T // 4), T // 4), :]) for i in range(7)]
        for c in range(0, F // 2, 128):
            gate, up = matmul(lambda i: lhs[i], wg, c), matmul(lambda i: lhs[i], wu, c)
            for i, term in enumerate(_lhs_terms(*map(_geglu, gate, up))):
                act[i, :, c:c + 128] = _pack(term)
        nxt = jnp.minimum(t + 1, NT - 1)
        norm(hs, nxt * T, T, halves, hn, (nxt + 1) * (T // 4), t < 0, L2)
        for c in range(0, D // 2, 128):
            for r, half, val in _row_groups(matmul(lambda i: _unpack(act[i]), wd, c)):
                cols = pl.ds(half * D // 2 + c, 128)
                xs[_ds(t * T + r, G // 2), cols] = (hs[_ds(T + t * T + r, G // 2), cols] + val).astype(BF16)
        cp_out(t).start()

    @_loop('drain', NT)
    def _(t):
        cp_out(t).wait()


@jax.jit
def pallas_sequential_preLN__sliding_local_dilated__glu_gated_geglu__prompt_kernel(
        A_x, A_wqkv, A_wo, B_x, B_w_gate, B_w_up, B_w_down):
    del B_x
    cfg = dict(CFG)
    flags = cfg.pop("FLAGS")
    any_spec = pl.BlockSpec(memory_space=pl.ANY)
    out = pl.pallas_call(
        functools.partial(_kernel, **cfg),
        in_specs=[any_spec] * 6,
        out_specs=any_spec,
        out_shape=jax.ShapeDtypeStruct((S, D), A_x.dtype),
        scratch_shapes=[
            pltpu.VMEM((S, D), BF16),
            pltpu.VMEM((3 * D, D), BF16),
            pltpu.VMEM((D, D), BF16),
            pltpu.VMEM((7, D // 4, D // 2), U32),
            pltpu.VMEM((7, D // 2, D // 2), U32),
            pltpu.VMEM((7, D // 4, D // 2), U32),
            pltpu.VMEM((D, F), BF16),
            pltpu.VMEM((D, F), BF16),
            pltpu.VMEM((F, D), BF16),
            pltpu.VMEM((H * ST, 128), U32),
            pltpu.VMEM((2, H * 9, 128), U32),
            pltpu.VMEM((7, S // 4, D // 2), U32),
            pltpu.VMEM((2 * NJ, P0 + S, 128), F32),
            pltpu.VMEM((NJ, P0 + S, 128), F32),
            pltpu.VMEM((W, T + 8, 128), F32),
            pltpu.VMEM((T + S, D), F32),
            pltpu.VMEM((T + S, D), F32),
            pltpu.VMEM((7, (T + S) // 4, D // 2), U32),
            pltpu.VMEM((7, T // 4, F // 2), U32),
            pltpu.SemaphoreType.DMA((NT,)),
            pltpu.SemaphoreType.DMA((3 * NS,)),
            pltpu.SemaphoreType.DMA((NJ,)),
            pltpu.SemaphoreType.DMA((3,)),
            pltpu.SemaphoreType.DMA((NT,)),
        ],
        compiler_params=pltpu.CompilerParams(vmem_limit_bytes=120 * 1024 * 1024, flags=flags),
    )(A_x.reshape(S, D), A_wqkv, A_wo, B_w_gate, B_w_up, B_w_down)
    return out.reshape(A_x.shape)
```

```python
import functools
import math

import jax
import jax.numpy as jnp
from jax import lax
import jax.experimental.pallas as pl
import jax.experimental.pallas.tpu as pltpu

CFG = dict(CJ=range(8), RQ=8, CH=2, PR=1, CM=range(8), CJW=range(8), CMW=range(8), TT=(0,), KJ='0202020201010101', KD=(6,27), OD=(6,12), FD=(300,400), CS=(0,-1,0,1,-1,2,1), ORD=(1,3,6,4,0,2,5), NW=128, SC=0, FLAGS=None)

S, D, F = 2048, 1024, 3584
H, DH, W, DIL = 32, 32, 8, 2
T = 256
NT = S // T
NS = D // T
NJ = D // 128
HALO = 16
P0 = T + HALO
ST = DH + 1
G = 32
ORDER = (1, 3, 6, 4, 0, 2, 5)
F32, BF16, U32 = jnp.float32, jnp.bfloat16, jnp.uint32


def _ln(x):
    m = jnp.mean(x, axis=-1, keepdims=True)
    c = x - m
    v = jnp.mean(c * c, axis=-1, keepdims=True)
    return c * lax.rsqrt(v + 1e-5)


def _geglu(g, u):
    c0 = math.sqrt(2.0 / math.pi)
    z = g * (c0 + (c0 * 0.044715) * (g * g))
    hg = 0.5 * g
    return (hg + hg * jnp.tanh(z)) * u


def _ds(start, size, align=None):
    if isinstance(start, int):
        return pl.ds(start, size)
    return pl.ds(pl.multiple_of(start, align or size), size)


def _tile(j):
    return slice(j * 128, (j + 1) * 128)


def _pack(x):
    return pltpu.bitcast(x.astype(BF16), U32)


def _unpack(x):
    return pltpu.bitcast(x, BF16)


def _lhs_terms(a11, a12, a21, a22):
    return a11 + a22, a21 + a22, a11, a22, a11 + a12, a21 - a11, a12 - a22


def _rhs_terms(b11, b12, b21, b22):
    f11, f12, f21, f22 = (b.astype(F32) for b in (b11, b12, b21, b22))
    return f11 + f22, b11, f12 - f22, f21 - f11, b22, f11 + f12, f21 + f22


def _strassen(lhs, rhs):
    m = {i: jnp.dot(lhs(i), rhs(i), preferred_element_type=F32) for i in CFG['ORD']}
    return m[3] + m[6] - m[4] + m[0], m[4] + m[2], m[1] + m[3], m[0] - m[1] + m[2] + m[5]


def _row_groups(c):
    n = G // 2
    return [(i * G + q // 2 * n, q % 2, c[q][i * n:(i + 1) * n]) for q in range(4) for i in range(T // G)]


def _even_odd(y):
    return [jnp.concatenate([y[:, _tile(j)] for j in range(e, NJ, 2)], axis=1) for e in range(2)]


def _loop(name, n):
    def deco(f):
        def g(t):
            if CFG["SC"]:
                with jax.named_scope(name):
                    f(t)
            else:
                f(t)
        pl.loop(0, n)(g)
    return deco


def _kernel(x_hbm, wqkv_hbm, wo_hbm, wg_hbm, wu_hbm, wd_hbm, out_hbm,
            xs, raw, raw_o, wk, wqv, wo, wg, wu, wd, tmp_c, tmp_r, xn, qv, ks, ps, os, hs, hn, act,
            sem_x, sem_w, sem_o, sem_f, sem_out, *, CJ, RQ, CH, PR, CM, CJW, CMW, TT, KJ, KD, OD, FD, CS, ORD, NW, SC):
    def cp_x(t):
        return pltpu.make_async_copy(x_hbm.at[_ds(t * T, T), :], xs.at[_ds(t * T, T), :], sem_x.at[t])

    def cp_w(u):
        col = jnp.where(u < NS, 1, u // NS * 2 - 2) if not isinstance(u, int) else (1, 0, 2)[u // NS]
        return pltpu.make_async_copy(wqkv_hbm.at[_ds(u % NS * T, T), _ds(col * D, D)],
                                     raw.at[_ds(u * T, T), :], sem_w.at[u])

    def cp_o(j):
        return pltpu.make_async_copy(wo_hbm.at[:, _ds(j * 128, 128)], raw_o.at[:, _ds(j * 128, 128)], sem_o.at[j])

    cp_ffn = [pltpu.make_async_copy(src, dst, sem_f.at[i])
              for i, (src, dst) in enumerate(((wg_hbm, wg), (wu_hbm, wu), (wd_hbm, wd)))]

    def cp_out(t):
        return pltpu.make_async_copy(xs.at[_ds(t * T, T), :], out_hbm.at[_ds(t * T, T), :], sem_out.at[t])

    def prepare_cols(u, dst, s):
        cols = pltpu.bitcast(raw[_ds(u * T, T), :], U32).T
        for h in range(H):
            tmp_c[h * ST:h * ST + DH, :] = cols[h * DH:(h + 1) * DH]

        def tile(j):
            rows = [tmp_c[pl.ds(4 * j + e, H, stride=ST), :] for e in range(4)]
            return _unpack(jnp.concatenate(rows, axis=0).T)

        for j in range(NJ // 2):
            left, right = tile(j), tile(j + NJ // 2)
            for i, term in enumerate(_rhs_terms(left[:128], right[:128], left[128:], right[128:])):
                dst[i, _ds(s * 64, 64), _tile(j)] = _pack(term)
            yield _pack(term)[-8:]

    def prepare_rows(j, half):
        for e in range(2):
            for h in range(H):
                rows = raw_o[_ds(h * DH + half * (DH // 2), DH // 2), _ds((j + e * NJ // 2) * 128, 128)]
                tmp_r[e, h * 9:h * 9 + 8, :] = pltpu.bitcast(rows, U32)
        for d in (0, 1, 2, 3, 8, 9, 10, 11):
            words = [tmp_r[e, pl.ds((d + k) // 2, H, stride=9), :] for k in (0, 4) for e in range(2)]
            quads = [pltpu.bitcast(w >> 16 << 16 if d % 2 else w << 16, F32) for w in words]
            for i, term in enumerate(_rhs_terms(*quads)):
                wo[i, _ds(half * 128 + (d // 8 * 4 + d % 8) * 16, 16), _ds(j * 128, 128)] = _pack(term)
            if d % 2:
                yield _pack(term)[-8:]

    def norm(src, base, off, split, dst, dbase, doff, n=T):
        for g in range(n // G):
            y = _ln(src[_ds(base + (off + g * G), G), :].astype(F32))
            terms = [_pack(a) for a in _lhs_terms(*split(y[:G // 2]), *split(y[G // 2:]))]
            for i, term in enumerate(terms):
                for j in range(NJ // 2):
                    dst[i * NJ // 2 + j, _ds(dbase + (doff + g * G // 4), G // 4), :] = term[:, _tile(j)]
            yield functools.reduce(jnp.bitwise_or, [terms[i][:, _tile(j)] for i in TT for j in range(NJ // 2)])

    def normed(src, quarter):
        return lambda i: _unpack(jnp.concatenate(
            [src[i * NJ // 2 + j, _ds(quarter, T // 4), :] for j in range(NJ // 2)], axis=1))

    def due(never, toks, first, last):
        calls = iter(range(1 << 20))

        def f(w):
            n = next(calls)
            for i, tok in enumerate(toks):
                if first + i * (last - first) // max(len(toks) - 1, 1) == n:
                    w = jnp.concatenate([jnp.where(never, tok, w[:8]), w[8:]], axis=0)
            return w
        return f

    def halves(y):
        return y[:, :D // 2], y[:, D // 2:]

    def windows(ref, j, base, row, n):
        blk = [ref[j, pl.ds(base + (row - 8 - DIL * w), n + 8), :] for w in range(W // 2)]
        return [b[8:] for b in blk] + [b[:n] for b in blk]

    def attend(base, off, n, zero, maybe_first, links_qk, links_pv):
        def fold(vals):
            return functools.reduce(jnp.maximum, [v[i:i + 8] for v in vals for i in range(0, v.shape[0], 8)])

        def logits(r):
            ls = None
            for j in range(NJ):
                q = qv[j, _ds(base + (P0 + off + r), RQ), :]
                pr = [q * k for k in windows(ks, j, zero + base, P0 + off + r, RQ)]
                ls = pr if ls is None else [l + p for l, p in zip(ls, pr)]
                if j in links_qk:
                    ks[0, 0:8, :] = fold([ls[(j + i * W // CH) % W] for i in range(CH)])
            return ls

        def softmax(r, ls):
            ls = [l + pltpu.roll(l, 64, 1) for l in ls]
            ls = [l + pltpu.roll(l, 32, 1) for l in ls]
            if maybe_first and r < HALO:
                pos = base + (off + r) + lax.broadcasted_iota(jnp.int32, (RQ, 128), 0)
                ls = [jnp.where(pos >= DIL * w, l, -1e9 * DH ** 0.5) for w, l in enumerate(ls)]
            m = functools.reduce(jnp.maximum, ls)
            es = [jnp.exp2((l - m) * (DH ** -0.5 * math.log2(math.e))) for l in ls]
            inv = 1.0 / functools.reduce(jnp.add, es)
            for w in range(W):
                ps[w, r:r + RQ, :] = es[w] * inv

        def mix(r):
            p = None
            for j in range(NJ):
                p = [ps[w, _ds(zero + r, 16), :] if p is None or (j - 1 in links_pv and w < PR) else p[w] for w in range(W)]
                acc = functools.reduce(jnp.add, [a * v for a, v in zip(p, windows(qv, NJ + j, base, P0 + off + r, 16))])
                os[_ds(base + (T + off + r), 16), _tile(j)] = acc
                if j in links_pv:
                    tok = fold([acc])
                    ps[0, T:T + 8, :] = tok
            return tok

        pending = []
        for r in range(0, n + 32, 16):
            new = [(r + i, logits(r + i)) for i in range(0, 16, RQ)] if r < n else []
            if new:
                ps[0, T:T + 8, :] = new[-1][1][NJ - 1][-8:]
            if r >= 32:
                ks[0, 0:8, :] = mix(r - 32)
            for job in pending:
                softmax(*job)
            pending = new

    def start_step(t):
        cp_x(t + 1).start()
        cp_w(NS + t).start()

    cp_w(0).start()
    cp_w(1).start()
    cp_o(0).start()
    cp_o(NJ // 2).start()
    for ref in (qv, ks):
        ref[:, 0:P0, :] = jnp.zeros((ref.shape[0], P0, 128), F32)
    hs[T:T + T // 4, :] = jnp.zeros((T // 4, D), F32)

    @_loop('perm', NS)
    def _(s):
        cp_w(s).wait()
        for i, start in enumerate((cp_w(2).start, cp_w(3).start, cp_x(0).start, lambda: start_step(0))):
            pl.when(s == i)(start)
        list(prepare_cols(s, wk, s))

    cp_x(0).wait()
    list(norm(xs, 0, 0, _even_odd, xn, 0, 0))
    start_step(1)

    def project(quarter, base, w, k0, out, plane, gate=lambda w: w):
        for c in range(0, D // 2, NW):
            res = _strassen(normed(xn, quarter),
                            lambda i: _unpack(gate(w[i, k0:k0 + D // 4, c:c + NW])))
            for r, half, val in _row_groups(res):
                for j in range(NW // 128):
                    out[plane + half * NJ // 2 + c // 128 + j, _ds(base + (P0 + r), G // 2), :] = val[:, _tile(j)]

    @_loop('K', NT)
    def _(t):
        pl.when(t + 1 < NT)(lambda: cp_x(t + 1).wait())
        cp_w(NS + t).wait()

        @pl.when(t % 2 == 0)
        def _():
            cp_o(t // 2).wait()
            cp_o(t // 2 + NJ // 2).wait()

            @pl.when(t + 2 < NT)
            def _():
                cp_o(t // 2 + 1).start()
                cp_o(t // 2 + 1 + NJ // 2).start()

        pl.when(t + 3 < NT)(lambda: cp_x(t + 3).start())
        pl.when(t + 2 < NT)(lambda: cp_w(NS + t + 2).start())

        @pl.when(t == NT - 2)
        def _():
            for c in cp_ffn:
                c.start()

        quarter = pl.multiple_of(t * (T // 4), T // 4)
        nxt = jnp.minimum(t + 1, NT - 1)
        jobs = (list(norm(xs, nxt * T, 0, _even_odd, xn, quarter, T // 4)), list(prepare_cols(NS + t, wqv, t)),
                list(prepare_rows(t // 2, t % 2)))
        project(quarter, t * T, wk, 0, ks, 0, due(t < 0, [jobs[int(c)].pop(0) for c in KJ], *KD))

    @_loop('QV', NT)
    def _(t):
        @pl.when(t == 1)
        def _():
            for j in range(NJ, 2 * NJ):
                qv[j, T:P0, :] = jnp.broadcast_to(qv[j, P0:P0 + 1, :], (HALO, 128))

        base = pl.multiple_of(t * T, T)
        attend(base, -T, T, pl.multiple_of(jnp.minimum(t, 0), T), True, CJ, CM)
        quarter = pl.multiple_of(t * (T // 4), T // 4)
        project(quarter, base, wqv, 0, qv, 0)
        project(quarter, base, wqv, D // 4, qv, NJ)

    @_loop('O', NT)
    def _(t):
        zero = pl.multiple_of(jnp.minimum(t, 0), T)
        base = pl.multiple_of(t * T, T)
        part = jnp.clip(t - 1, 0, 3) * (T // 4)
        gate = due(t < 0, list(norm(hs, part, T, halves, hn, part // 4, 0, n=T // 4)), *OD)
        blocks = [jnp.concatenate([os[_ds(T + t * T + g * G + e * G // 2, G // 2), :] for g in range(T // G)], axis=0)
                  for e in range(2)]
        lhs = [a.astype(BF16) for a in _lhs_terms(*_even_odd(blocks[0]), *_even_odd(blocks[1]))]
        attend(pl.multiple_of(jnp.minimum(t * 48, T - 48), 16), S - T, 48, zero, False, CJW, CMW)
        for c in range(0, D // 2, NW):
            res = _strassen(lambda i: lhs[i], lambda i: _unpack(gate(wo[i, :, c:c + NW])))
            for r, half, val in _row_groups(res):
                cols = pl.ds(half * D // 2 + c, NW)
                hs[_ds(base + (T + r), G // 2), cols] = xs[_ds(base + r, G // 2), cols].astype(F32) + val

    for c in cp_ffn:
        c.wait()

    @_loop('FFN', NT)
    def _(t):
        def matmul(lhs, w, c):
            k2, n2 = w.shape[0] // 2, w.shape[1] // 2

            def rhs(i):
                z = jnp.minimum(t, -CS[i]) + CS[i] if CS[i] >= 0 else 0
                return _rhs_terms(*(w[_ds(z + r, k2, 128), j + c:j + c + 128] for r in (0, k2) for j in (0, n2)))[i]
            return _strassen(lhs, lambda i: _unpack(wait(_pack(rhs(i)))))

        quarter = pl.multiple_of(t * (T // 4), T // 4)
        lhs = normed(hn, quarter)
        nxt = jnp.minimum(t + 1, NT - 1)
        wait = due(t < 0, list(norm(hs, nxt * T, T, halves, hn, quarter, T // 4)), *FD)
        for c in range(0, F // 2, 128):
            gate, up = matmul(lhs, wg, c), matmul(lhs, wu, c)
            for i, term in enumerate(_lhs_terms(*map(_geglu, gate, up))):
                act[i, :, c:c + 128] = _pack(term)
        for c in range(0, D // 2, 128):
            for r, half, val in _row_groups(matmul(lambda i: _unpack(act[i]), wd, c)):
                cols = pl.ds(half * D // 2 + c, 128)
                xs[_ds(t * T + r, G // 2), cols] = (hs[_ds(T + t * T + r, G // 2), cols] + val).astype(BF16)
        cp_out(t).start()

    @_loop('drain', NT)
    def _(t):
        cp_out(t).wait()


@jax.jit
def pallas_sequential_preLN__sliding_local_dilated__glu_gated_geglu__prompt_kernel(
        A_x, A_wqkv, A_wo, B_x, B_w_gate, B_w_up, B_w_down):
    del B_x
    cfg = dict(CFG)
    flags = cfg.pop("FLAGS")
    any_spec = pl.BlockSpec(memory_space=pl.ANY)
    out = pl.pallas_call(
        functools.partial(_kernel, **cfg),
        in_specs=[any_spec] * 6,
        out_specs=any_spec,
        out_shape=jax.ShapeDtypeStruct((S, D), A_x.dtype),
        scratch_shapes=[
            pltpu.VMEM((S, D), BF16),
            pltpu.VMEM((3 * D, D), BF16),
            pltpu.VMEM((D, D), BF16),
            pltpu.VMEM((7, D // 4, D // 2), U32),
            pltpu.VMEM((7, D // 2, D // 2), U32),
            pltpu.VMEM((7, D // 4, D // 2), U32),
            pltpu.VMEM((D, F), BF16),
            pltpu.VMEM((D, F), BF16),
            pltpu.VMEM((F, D), BF16),
            pltpu.VMEM((H * ST, 128), U32),
            pltpu.VMEM((2, H * 9, 128), U32),
            pltpu.VMEM((7 * NJ // 2, (S + T) // 4, 128), U32),
            pltpu.VMEM((2 * NJ, P0 + S, 128), F32),
            pltpu.VMEM((NJ, P0 + S, 128), F32),
            pltpu.VMEM((W, T + 8, 128), F32),
            pltpu.VMEM((T + S, D), F32),
            pltpu.VMEM((T + S, D), F32),
            pltpu.VMEM((7 * NJ // 2, (S + T) // 4, 128), U32),
            pltpu.VMEM((7, T // 4, F // 2), U32),
            pltpu.SemaphoreType.DMA((NT,)),
            pltpu.SemaphoreType.DMA((3 * NS,)),
            pltpu.SemaphoreType.DMA((NJ,)),
            pltpu.SemaphoreType.DMA((3,)),
            pltpu.SemaphoreType.DMA((NT,)),
        ],
        compiler_params=pltpu.CompilerParams(vmem_limit_bytes=120 * 1024 * 1024, flags=flags),
    )(A_x.reshape(S, D), A_wqkv, A_wo, B_w_gate, B_w_up, B_w_down)
    return out.reshape(A_x.shape)
```

```python
import functools
import math

import jax
import jax.numpy as jnp
from jax import lax
import jax.experimental.pallas as pl
import jax.experimental.pallas.tpu as pltpu

CFG = dict(CJ=range(8), RQ=8, CH=8, PR=1, CM=range(8), CJW=range(8), CMW=range(8), TT=(0,), KJ='000101010100', RA=(0,3), OP=64, KD=(8,27), OD=(6,12), FD=(300,400), CS=(0,-1,0,1,-1,2,1), ORD=(1,3,6,4,0,2,5), NW=128, SC=0, FLAGS=None)

S, D, F = 2048, 1024, 3584
H, DH, W, DIL = 32, 32, 8, 2
T = 256
NT = S // T
NS = D // T
NJ = D // 128
HALO = 16
P0 = T + HALO
ST = DH + 1
G = 32
ORDER = (1, 3, 6, 4, 0, 2, 5)
F32, BF16, U32 = jnp.float32, jnp.bfloat16, jnp.uint32


def _ln(x):
    m = jnp.mean(x, axis=-1, keepdims=True)
    c = x - m
    v = jnp.mean(c * c, axis=-1, keepdims=True)
    return c * lax.rsqrt(v + 1e-5)


def _geglu(g, u):
    c0 = math.sqrt(2.0 / math.pi)
    z = g * (c0 + (c0 * 0.044715) * (g * g))
    hg = 0.5 * g
    return (hg + hg * jnp.tanh(z)) * u


def _ds(start, size, align=None):
    if isinstance(start, int):
        return pl.ds(start, size)
    return pl.ds(pl.multiple_of(start, align or size), size)


def _tile(j):
    return slice(j * 128, (j + 1) * 128)


def _pack(x):
    return pltpu.bitcast(x.astype(BF16), U32)


def _unpack(x):
    return pltpu.bitcast(x, BF16)


def _lhs_terms(a11, a12, a21, a22):
    return a11 + a22, a21 + a22, a11, a22, a11 + a12, a21 - a11, a12 - a22


def _rhs_terms(b11, b12, b21, b22):
    f11, f12, f21, f22 = (b.astype(F32) for b in (b11, b12, b21, b22))
    return f11 + f22, b11, f12 - f22, f21 - f11, b22, f11 + f12, f21 + f22


def _strassen(lhs, rhs):
    m = {i: jnp.dot(lhs(i), rhs(i), preferred_element_type=F32) for i in CFG['ORD']}
    return m[3] + m[6] - m[4] + m[0], m[4] + m[2], m[1] + m[3], m[0] - m[1] + m[2] + m[5]


def _row_groups(c):
    n = G // 2
    return [(i * G + q // 2 * n, q % 2, c[q][i * n:(i + 1) * n]) for q in range(4) for i in range(T // G)]


def _even_odd(y):
    return [jnp.concatenate([y[:, _tile(j)] for j in range(e, NJ, 2)], axis=1) for e in range(2)]


def _loop(name, n):
    def deco(f):
        def g(t):
            if CFG["SC"]:
                with jax.named_scope(name):
                    f(t)
            else:
                f(t)
        pl.loop(0, n)(g)
    return deco


def _kernel(x_hbm, wqkv_hbm, wo_hbm, wg_hbm, wu_hbm, wd_hbm, out_hbm,
            xs, raw, raw_o, wk, wqv, wo, wg, wu, wd, tmp_c, tmp_r, xn, qv, ks, ps, os, hs, hn, act,
            sem_x, sem_w, sem_o, sem_f, sem_out, *, CJ, RQ, CH, PR, CM, CJW, CMW, TT, RA, OP, KJ, KD, OD, FD, CS, ORD, NW, SC):
    def cp_x(t):
        return pltpu.make_async_copy(x_hbm.at[_ds(t * T, T), :], xs.at[_ds(t * T, T), :], sem_x.at[t])

    def cp_w(u):
        col = jnp.where(u < NS, 1, u // NS * 2 - 2) if not isinstance(u, int) else (1, 0, 2)[u // NS]
        return pltpu.make_async_copy(wqkv_hbm.at[_ds(u % NS * T, T), _ds(col * D, D)],
                                     raw.at[_ds(u * T, T), :], sem_w.at[u])

    cp_o = pltpu.make_async_copy(wo_hbm, raw_o, sem_o)
    cp_ffn = [pltpu.make_async_copy(src, dst, sem_f.at[i])
              for i, (src, dst) in enumerate(((wg_hbm, wg), (wu_hbm, wu), (wd_hbm, wd)))]

    def cp_out(t):
        return pltpu.make_async_copy(xs.at[_ds(t * T, T), :], out_hbm.at[_ds(t * T, T), :], sem_out.at[t])

    def prepare_cols(u, dst, s):
        cols = pltpu.bitcast(raw[_ds(u * T, T), :], U32).T
        for h in range(H):
            tmp_c[h * ST:h * ST + DH, :] = cols[h * DH:(h + 1) * DH]

        def tile(j):
            rows = [tmp_c[pl.ds(4 * j + e, H, stride=ST), :] for e in range(4)]
            return _unpack(jnp.concatenate(rows, axis=0).T)

        for j in range(NJ // 2):
            left, right = tile(j), tile(j + NJ // 2)
            for i, term in enumerate(_rhs_terms(left[:128], right[:128], left[128:], right[128:])):
                dst[i, _ds(s * 64, 64), _tile(j)] = _pack(term)
            yield _pack(term)[-8:]

    def prepare_rows(j, half, after):
        for e in range(2):
            for h in range(H):
                rows = raw_o[_ds(h * DH + half * (DH // 2), DH // 2), _ds((j + e * NJ // 2) * 128, 128)]
                tmp_r[e, h * 9:h * 9 + 8, :] = pltpu.bitcast(rows, U32)
        for d in (0, 1, 2, 3, 8, 9, 10, 11):
            words = [tmp_r[e, pl.ds((d + k) // 2, H, stride=9), :] for k in (0, 4) for e in range(2)]
            quads = [pltpu.bitcast(w >> 16 << 16 if d % 2 else w << 16, F32) for w in words]
            quads = [after(q) if i in RA else q for i, q in enumerate(quads)]
            for i, term in enumerate(_rhs_terms(*quads)):
                wo[i, _ds(half * 128 + (d // 8 * 4 + d % 8) * 16, 16), _ds(j * 128, 128)] = _pack(term)
            yield term

    def norm(src, base, off, split, dst, dbase, doff, n=T):
        for g in range(n // G):
            y = _ln(src[_ds(base + (off + g * G), G), :].astype(F32))
            terms = [_pack(a) for a in _lhs_terms(*split(y[:G // 2]), *split(y[G // 2:]))]
            for i, term in enumerate(terms):
                for j in range(NJ // 2):
                    dst[i * NJ // 2 + j, _ds(dbase + (doff + g * G // 4), G // 4), :] = term[:, _tile(j)]
            yield functools.reduce(jnp.bitwise_or, [terms[i][:, _tile(j)] for i in TT for j in range(NJ // 2)])

    def normed(src, quarter):
        return lambda i: _unpack(jnp.concatenate(
            [src[i * NJ // 2 + j, _ds(quarter, T // 4), :] for j in range(NJ // 2)], axis=1))

    def due(never, toks, first, last):
        calls = iter(range(1 << 20))

        def f(w):
            n = next(calls)
            for i, tok in enumerate(toks):
                if first + i * (last - first) // max(len(toks) - 1, 1) == n:
                    w = jnp.concatenate([jnp.where(never, tok, w[:8]), w[8:]], axis=0)
            return w
        return f

    def halves(y):
        return y[:, :D // 2], y[:, D // 2:]

    def windows(ref, j, base, row, n):
        blk = [ref[j, pl.ds(base + (row - 8 - DIL * w), n + 8), :] for w in range(W // 2)]
        return [b[8:] for b in blk] + [b[:n] for b in blk]

    def attend(base, off, n, zero, maybe_first, links_qk, links_pv, side=None):
        def fold(vals):
            return functools.reduce(jnp.maximum, [v[i:i + 8] for v in vals for i in range(0, v.shape[0], 8)])

        tok = [None]

        def after(x):
            if tok[0] is None:
                return x
            return jnp.where(zero < 0, jnp.concatenate([tok[0]] * (x.shape[0] // 8), axis=0), x)

        def logits(r):
            ls = None
            for j in range(NJ):
                q = after(qv[j, _ds(base + (P0 + off + r), RQ), :])
                pr = [q * k for k in windows(ks, j, base, P0 + off + r, RQ)]
                ls = pr if ls is None else [l + p for l, p in zip(ls, pr)]
                if j in links_qk:
                    tok[0] = fold([ls[(j + i * W // CH) % W] for i in range(CH)])
            return ls

        def softmax(r, ls):
            ls = [l + pltpu.roll(l, 64, 1) for l in ls]
            ls = [l + pltpu.roll(l, 32, 1) for l in ls]
            if maybe_first and r < HALO:
                pos = base + (off + r) + lax.broadcasted_iota(jnp.int32, (RQ, 128), 0)
                ls = [jnp.where(pos >= DIL * w, l, -1e9 * DH ** 0.5) for w, l in enumerate(ls)]
            m = functools.reduce(jnp.maximum, ls)
            es = [jnp.exp2((l - m) * (DH ** -0.5 * math.log2(math.e))) for l in ls]
            inv = 1.0 / functools.reduce(jnp.add, es)
            for w in range(W):
                ps[w, r:r + RQ, :] = es[w] * inv

        def mix(r):
            p = [ps[w, r:r + 16, :] for w in range(W)]
            for j in range(NJ):
                pj = [after(a) if w < PR else a for w, a in enumerate(p)]
                acc = functools.reduce(jnp.add, [a * v for a, v in zip(pj, windows(qv, NJ + j, base, P0 + off + r, 16))])
                os[_ds(base + (T + off + r), 16), _tile(j)] = acc
                if j in links_pv:
                    tok[0] = fold([acc])

        pending = []
        side = side and side(after)
        for r in range(0, n + 32, 16):
            if side and r % 32 == 16 and r < n:
                tok[0] = fold([next(side)])
            new = [(r + i, logits(r + i)) for i in range(0, 16, RQ)] if r < n else []
            if r >= 32:
                mix(r - 32)
            for job in pending:
                softmax(*job)
            pending = new

    def start_step(t):
        cp_x(t + 1).start()
        cp_w(NS + t).start()

    cp_w(0).start()
    cp_w(1).start()
    for ref in (qv, ks):
        ref[:, 0:P0, :] = jnp.zeros((ref.shape[0], P0, 128), F32)
    hs[T:T + T // 4, :] = jnp.zeros((T // 4, D), F32)

    @_loop('perm', NS)
    def _(s):
        cp_w(s).wait()
        for i, start in enumerate((cp_w(2).start, cp_w(3).start, cp_x(0).start, lambda: start_step(0))):
            pl.when(s == i)(start)
        list(prepare_cols(s, wk, s))

    cp_x(0).wait()
    list(norm(xs, 0, 0, _even_odd, xn, 0, 0))
    start_step(1)

    def project(quarter, base, w, k0, out, plane, gate=lambda w: w):
        for c in range(0, D // 2, NW):
            res = _strassen(normed(xn, quarter),
                            lambda i: _unpack(gate(w[i, k0:k0 + D // 4, c:c + NW])))
            for r, half, val in _row_groups(res):
                for j in range(NW // 128):
                    out[plane + half * NJ // 2 + c // 128 + j, _ds(base + (P0 + r), G // 2), :] = val[:, _tile(j)]

    @_loop('K', NT)
    def _(t):
        pl.when(t + 1 < NT)(lambda: cp_x(t + 1).wait())
        cp_w(NS + t).wait()

        pl.when(t + 3 < NT)(lambda: cp_x(t + 3).start())
        pl.when(t + 2 < NT)(lambda: cp_w(NS + t + 2).start())

        pl.when(t == NT - 2)(cp_o.start)

        quarter = pl.multiple_of(t * (T // 4), T // 4)
        nxt = jnp.minimum(t + 1, NT - 1)
        jobs = (list(norm(xs, nxt * T, 0, _even_odd, xn, quarter, T // 4)), list(prepare_cols(NS + t, wqv, t)))
        project(quarter, t * T, wk, 0, ks, 0, due(t < 0, [jobs[int(c)].pop(0) for c in KJ], *KD))

    cp_o.wait()
    for c in cp_ffn:
        c.start()

    @_loop('QV', NT)
    def _(t):
        @pl.when(t == 1)
        def _():
            for j in range(NJ, 2 * NJ):
                qv[j, T:P0, :] = jnp.broadcast_to(qv[j, P0:P0 + 1, :], (HALO, 128))

        base = pl.multiple_of(t * T, T)
        attend(base, -T, T, pl.multiple_of(jnp.minimum(t, 0), T), True, CJ, CM,
               functools.partial(prepare_rows, t // 2, t % 2))
        quarter = pl.multiple_of(t * (T // 4), T // 4)
        project(quarter, base, wqv, 0, qv, 0)
        project(quarter, base, wqv, D // 4, qv, NJ)

    @_loop('O', NT)
    def _(t):
        zero = pl.multiple_of(jnp.minimum(t, 0), T)
        base = pl.multiple_of(t * T, T)
        part = jnp.clip(t - 1, 0, 3) * (T // 4)
        gate = due(t < 0, list(norm(hs, part, T, halves, hn, part // 4, 0, n=T // 4)), *OD)
        blocks = [jnp.concatenate([os[_ds(T + t * T + g * G + e * G // 2, G // 2), :] for g in range(T // G)], axis=0)
                  for e in range(2)]
        lhs = [a.astype(BF16) for a in _lhs_terms(*_even_odd(blocks[0]), *_even_odd(blocks[1]))]
        attend(pl.multiple_of(jnp.minimum(t * OP, T - OP), 16), S - T, OP, zero, False, CJW, CMW)
        for c in range(0, D // 2, NW):
            res = _strassen(lambda i: lhs[i], lambda i: _unpack(gate(wo[i, :, c:c + NW])))
            for r, half, val in _row_groups(res):
                cols = pl.ds(half * D // 2 + c, NW)
                hs[_ds(base + (T + r), G // 2), cols] = xs[_ds(base + r, G // 2), cols].astype(F32) + val

    for c in cp_ffn:
        c.wait()

    @_loop('FFN', NT)
    def _(t):
        def matmul(lhs, w, c):
            k2, n2 = w.shape[0] // 2, w.shape[1] // 2

            def rhs(i):
                z = jnp.minimum(t, -CS[i]) + CS[i] if CS[i] >= 0 else 0
                return _rhs_terms(*(w[_ds(z + r, k2, 128), j + c:j + c + 128] for r in (0, k2) for j in (0, n2)))[i]
            return _strassen(lhs, lambda i: _unpack(wait(_pack(rhs(i)))))

        quarter = pl.multiple_of(t * (T // 4), T // 4)
        lhs = normed(hn, quarter)
        nxt = jnp.minimum(t + 1, NT - 1)
        wait = due(t < 0, list(norm(hs, nxt * T, T, halves, hn, quarter, T // 4)), *FD)
        for c in range(0, F // 2, 128):
            gate, up = matmul(lhs, wg, c), matmul(lhs, wu, c)
            for i, term in enumerate(_lhs_terms(*map(_geglu, gate, up))):
                act[i, :, c:c + 128] = _pack(term)
        for c in range(0, D // 2, 128):
            for r, half, val in _row_groups(matmul(lambda i: _unpack(act[i]), wd, c)):
                cols = pl.ds(half * D // 2 + c, 128)
                xs[_ds(t * T + r, G // 2), cols] = (hs[_ds(T + t * T + r, G // 2), cols] + val).astype(BF16)
        cp_out(t).start()

    @_loop('drain', NT)
    def _(t):
        cp_out(t).wait()


@jax.jit
def pallas_sequential_preLN__sliding_local_dilated__glu_gated_geglu__prompt_kernel(
        A_x, A_wqkv, A_wo, B_x, B_w_gate, B_w_up, B_w_down):
    del B_x
    cfg = dict(CFG)
    flags = cfg.pop("FLAGS")
    any_spec = pl.BlockSpec(memory_space=pl.ANY)
    out = pl.pallas_call(
        functools.partial(_kernel, **cfg),
        in_specs=[any_spec] * 6,
        out_specs=any_spec,
        out_shape=jax.ShapeDtypeStruct((S, D), A_x.dtype),
        scratch_shapes=[
            pltpu.VMEM((S, D), BF16),
            pltpu.VMEM((3 * D, D), BF16),
            pltpu.VMEM((D, D), BF16),
            pltpu.VMEM((7, D // 4, D // 2), U32),
            pltpu.VMEM((7, D // 2, D // 2), U32),
            pltpu.VMEM((7, D // 4, D // 2), U32),
            pltpu.VMEM((D, F), BF16),
            pltpu.VMEM((D, F), BF16),
            pltpu.VMEM((F, D), BF16),
            pltpu.VMEM((H * ST, 128), U32),
            pltpu.VMEM((2, H * 9, 128), U32),
            pltpu.VMEM((7 * NJ // 2, (S + T) // 4, 128), U32),
            pltpu.VMEM((2 * NJ, P0 + S, 128), F32),
            pltpu.VMEM((NJ, P0 + S, 128), F32),
            pltpu.VMEM((W, T + 8, 128), F32),
            pltpu.VMEM((T + S, D), F32),
            pltpu.VMEM((T + S, D), F32),
            pltpu.VMEM((7 * NJ // 2, (S + T) // 4, 128), U32),
            pltpu.VMEM((7, T // 4, F // 2), U32),
            pltpu.SemaphoreType.DMA((NT,)),
            pltpu.SemaphoreType.DMA((3 * NS,)),
            pltpu.SemaphoreType.DMA(()),
            pltpu.SemaphoreType.DMA((3,)),
            pltpu.SemaphoreType.DMA((NT,)),
        ],
        compiler_params=pltpu.CompilerParams(vmem_limit_bytes=120 * 1024 * 1024, flags=flags),
    )(A_x.reshape(S, D), A_wqkv, A_wo, B_w_gate, B_w_up, B_w_down)
    return out.reshape(A_x.shape)
```

```python
import functools
import math

import jax
import jax.numpy as jnp
from jax import lax
import jax.experimental.pallas as pl
import jax.experimental.pallas.tpu as pltpu

CFG = dict(CJ=[[i] for i in range(8)], RQ=8, CH=8, PR=1, CM=range(8), CJW=((0,4),(1,5),(2,6),(3,7)), CMW=range(8), TT=(0,), KJ='000101010100', RA=(0,3), OP=48, KD=(8,27), OD=(4,20), FD=(300,400), CS=(0,-1,0,1,-1,2,1), ORD=(1,3,6,4,0,2,5), NW=128, SC=0, FLAGS=None)

S, D, F = 2048, 1024, 3584
H, DH, W, DIL = 32, 32, 8, 2
T = 256
NT = S // T
NS = D // T
NJ = D // 128
HALO = 16
P0 = T + HALO
ST = DH + 1
G = 32
ORDER = (1, 3, 6, 4, 0, 2, 5)
F32, BF16, U32 = jnp.float32, jnp.bfloat16, jnp.uint32


def _ln(x):
    m = jnp.mean(x, axis=-1, keepdims=True)
    c = x - m
    v = jnp.mean(c * c, axis=-1, keepdims=True)
    return c * lax.rsqrt(v + 1e-5)


def _geglu(g, u):
    c0 = math.sqrt(2.0 / math.pi)
    z = g * (c0 + (c0 * 0.044715) * (g * g))
    hg = 0.5 * g
    return (hg + hg * jnp.tanh(z)) * u


def _ds(start, size, align=None):
    if isinstance(start, int):
        return pl.ds(start, size)
    return pl.ds(pl.multiple_of(start, align or size), size)


def _tile(j):
    return slice(j * 128, (j + 1) * 128)


def _pack(x):
    return pltpu.bitcast(x.astype(BF16), U32)


def _unpack(x):
    return pltpu.bitcast(x, BF16)


def _lhs_terms(a11, a12, a21, a22):
    return a11 + a22, a21 + a22, a11, a22, a11 + a12, a21 - a11, a12 - a22


def _rhs_terms(b11, b12, b21, b22):
    f11, f12, f21, f22 = (b.astype(F32) for b in (b11, b12, b21, b22))
    return f11 + f22, b11, f12 - f22, f21 - f11, b22, f11 + f12, f21 + f22


def _strassen(lhs, rhs):
    m = {i: jnp.dot(lhs(i), rhs(i), preferred_element_type=F32) for i in CFG['ORD']}
    return m[3] + m[6] - m[4] + m[0], m[4] + m[2], m[1] + m[3], m[0] - m[1] + m[2] + m[5]


def _row_groups(c):
    n = G // 2
    return [(i * G + q // 2 * n, q % 2, c[q][i * n:(i + 1) * n]) for q in range(4) for i in range(T // G)]


def _even_odd(y):
    return [jnp.concatenate([y[:, _tile(j)] for j in range(e, NJ, 2)], axis=1) for e in range(2)]


def _loop(name, n):
    def deco(f):
        def g(t):
            if CFG["SC"]:
                with jax.named_scope(name):
                    f(t)
            else:
                f(t)
        pl.loop(0, n)(g)
    return deco


def _kernel(x_hbm, wqkv_hbm, wo_hbm, wg_hbm, wu_hbm, wd_hbm, out_hbm,
            xs, raw, raw_o, wk, wqv, wo, wg, wu, wd, tmp_c, tmp_r, xn, qv, ks, ps, os, hs, hn, act,
            sem_x, sem_w, sem_o, sem_f, sem_out, *, CJ, RQ, CH, PR, CM, CJW, CMW, TT, RA, OP, KJ, KD, OD, FD, CS, ORD, NW, SC):
    def cp_x(t):
        return pltpu.make_async_copy(x_hbm.at[_ds(t * T, T), :], xs.at[_ds(t * T, T), :], sem_x.at[t])

    def cp_w(u):
        col = jnp.where(u < NS, 1, u // NS * 2 - 2) if not isinstance(u, int) else (1, 0, 2)[u // NS]
        return pltpu.make_async_copy(wqkv_hbm.at[_ds(u % NS * T, T), _ds(col * D, D)],
                                     raw.at[_ds(u * T, T), :], sem_w.at[u])

    cp_o = pltpu.make_async_copy(wo_hbm, raw_o, sem_o)
    cp_ffn = [pltpu.make_async_copy(src, dst, sem_f.at[i])
              for i, (src, dst) in enumerate(((wg_hbm, wg), (wu_hbm, wu), (wd_hbm, wd)))]

    def cp_out(t):
        return pltpu.make_async_copy(xs.at[_ds(t * T, T), :], out_hbm.at[_ds(t * T, T), :], sem_out.at[t])

    def prepare_cols(u, dst, s):
        cols = pltpu.bitcast(raw[_ds(u * T, T), :], U32).T
        for h in range(H):
            tmp_c[h * ST:h * ST + DH, :] = cols[h * DH:(h + 1) * DH]

        def tile(j):
            rows = [tmp_c[pl.ds(4 * j + e, H, stride=ST), :] for e in range(4)]
            return _unpack(jnp.concatenate(rows, axis=0).T)

        for j in range(NJ // 2):
            left, right = tile(j), tile(j + NJ // 2)
            for i, term in enumerate(_rhs_terms(left[:128], right[:128], left[128:], right[128:])):
                dst[i, _ds(s * 64, 64), _tile(j)] = _pack(term)
            yield _pack(term)[-8:]

    def prepare_rows(j, half, after):
        for e in range(2):
            for h in range(H):
                rows = raw_o[_ds(h * DH + half * (DH // 2), DH // 2), _ds((j + e * NJ // 2) * 128, 128)]
                tmp_r[e, h * 9:h * 9 + 8, :] = pltpu.bitcast(rows, U32)
        for d in (0, 1, 2, 3, 8, 9, 10, 11):
            words = [tmp_r[e, pl.ds((d + k) // 2, H, stride=9), :] for k in (0, 4) for e in range(2)]
            quads = [pltpu.bitcast(w >> 16 << 16 if d % 2 else w << 16, F32) for w in words]
            quads = [after(q) if i in RA else q for i, q in enumerate(quads)]
            for i, term in enumerate(_rhs_terms(*quads)):
                wo[i, _ds(half * 128 + (d // 8 * 4 + d % 8) * 16, 16), _ds(j * 128, 128)] = _pack(term)
            yield term

    def norm(src, base, off, split, dst, dbase, doff, n=T):
        for g in range(n // G):
            rows = _ds(base + (off + g * G), G)
            y = _ln(src[rows, :].astype(F32) if src is xs else
                    jnp.concatenate([src[j, rows, :] for j in range(NJ)], axis=1))
            terms = [_pack(a) for a in _lhs_terms(*split(y[:G // 2]), *split(y[G // 2:]))]
            for i, term in enumerate(terms):
                for j in range(NJ // 2):
                    dst[i * NJ // 2 + j, _ds(dbase + (doff + g * G // 4), G // 4), :] = term[:, _tile(j)]
            yield functools.reduce(jnp.bitwise_or, [terms[i][:, _tile(j)] for i in TT for j in range(NJ // 2)])

    def normed(src, quarter):
        return lambda i: _unpack(jnp.concatenate(
            [src[i * NJ // 2 + j, _ds(quarter, T // 4), :] for j in range(NJ // 2)], axis=1))

    def due(never, toks, first, last):
        calls = iter(range(1 << 20))

        def f(w):
            n = next(calls)
            for i, tok in enumerate(toks):
                if first + i * (last - first) // max(len(toks) - 1, 1) == n:
                    w = jnp.concatenate([jnp.where(never, tok, w[:8]), w[8:]], axis=0)
            return w
        return f

    def halves(y):
        return y[:, :D // 2], y[:, D // 2:]

    def windows(ref, j, base, row, n):
        blk = [ref[j, pl.ds(base + (row - 8 - DIL * w), n + 8), :] for w in range(W // 2)]
        return [b[8:] for b in blk] + [b[:n] for b in blk]

    def attend(base, off, n, zero, maybe_first, links_qk, links_pv, side=None):
        def fold(vals):
            return functools.reduce(jnp.maximum, [v[i:i + 8] for v in vals for i in range(0, v.shape[0], 8)])

        tok = [None]

        def after(x):
            if tok[0] is None:
                return x
            return jnp.where(zero < 0, jnp.concatenate([tok[0]] * (x.shape[0] // 8), axis=0), x)

        def logits(r):
            qs = [qv[j, _ds(base + (P0 + off + r), RQ), :] for j in range(NJ)]
            kw = [windows(ks, j, base, P0 + off + r, RQ) for j in range(NJ)]
            ls = {}
            for group in links_qk:
                first = after(qs[0])
                for w in group:
                    ls[w] = functools.reduce(jnp.add, [q * k[w] for q, k in zip([first] + qs[1:], kw)])
                tok[0] = fold([ls[w] for w in group])
            return [ls[w] for w in range(W)]

        def softmax(r, ls):
            ls = [l + pltpu.roll(l, 64, 1) for l in ls]
            ls = [l + pltpu.roll(l, 32, 1) for l in ls]
            if maybe_first and r < HALO:
                pos = base + (off + r) + lax.broadcasted_iota(jnp.int32, (RQ, 128), 0)
                ls = [jnp.where(pos >= DIL * w, l, -1e9 * DH ** 0.5) for w, l in enumerate(ls)]
            m = functools.reduce(jnp.maximum, ls)
            es = [jnp.exp2((l - m) * (DH ** -0.5 * math.log2(math.e))) for l in ls]
            inv = 1.0 / functools.reduce(jnp.add, es)
            for w in range(W):
                ps[w, r:r + RQ, :] = es[w] * inv

        def mix(r):
            p = [ps[w, r:r + 16, :] for w in range(W)]
            for j in range(NJ):
                pj = [after(a) if w < PR else a for w, a in enumerate(p)]
                acc = functools.reduce(jnp.add, [a * v for a, v in zip(pj, windows(qv, NJ + j, base, P0 + off + r, 16))])
                os[_ds(base + (T + off + r), 16), _tile(j)] = acc
                if j in links_pv:
                    tok[0] = fold([acc])

        pending = []
        side = side and side(after)
        for r in range(0, n + 32, 16):
            if side and r % 32 == 16 and r < n:
                tok[0] = fold([next(side)])
            new = [(r + i, logits(r + i)) for i in range(0, 16, RQ)] if r < n else []
            if r >= 32:
                mix(r - 32)
            for job in pending:
                softmax(*job)
            pending = new

    def start_step(t):
        cp_x(t + 1).start()
        cp_w(NS + t).start()

    cp_w(0).start()
    cp_w(1).start()
    for ref in (qv, ks):
        ref[:, 0:P0, :] = jnp.zeros((ref.shape[0], P0, 128), F32)
    hs[:, 0:T, :] = jnp.zeros((NJ, T, 128), F32)

    @_loop('perm', NS)
    def _(s):
        cp_w(s).wait()
        for i, start in enumerate((cp_w(2).start, cp_w(3).start, cp_x(0).start, lambda: start_step(0))):
            pl.when(s == i)(start)
        list(prepare_cols(s, wk, s))

    cp_x(0).wait()
    list(norm(xs, 0, 0, _even_odd, xn, 0, 0))
    start_step(1)

    def project(quarter, base, w, k0, out, plane, gate=lambda w: w):
        for c in range(0, D // 2, NW):
            res = _strassen(normed(xn, quarter),
                            lambda i: _unpack(gate(w[i, k0:k0 + D // 4, c:c + NW])))
            for r, half, val in _row_groups(res):
                for j in range(NW // 128):
                    out[plane + half * NJ // 2 + c // 128 + j, _ds(base + (P0 + r), G // 2), :] = val[:, _tile(j)]

    @_loop('K', NT)
    def _(t):
        pl.when(t + 1 < NT)(lambda: cp_x(t + 1).wait())
        cp_w(NS + t).wait()

        pl.when(t + 3 < NT)(lambda: cp_x(t + 3).start())
        pl.when(t + 2 < NT)(lambda: cp_w(NS + t + 2).start())

        pl.when(t == NT - 2)(cp_o.start)

        quarter = pl.multiple_of(t * (T // 4), T // 4)
        nxt = jnp.minimum(t + 1, NT - 1)
        jobs = (list(norm(xs, nxt * T, 0, _even_odd, xn, quarter, T // 4)), list(prepare_cols(NS + t, wqv, t)))
        project(quarter, t * T, wk, 0, ks, 0, due(t < 0, [jobs[int(c)].pop(0) for c in KJ], *KD))

    cp_o.wait()
    for c in cp_ffn:
        c.start()

    @_loop('QV', NT)
    def _(t):
        @pl.when(t == 1)
        def _():
            for j in range(NJ, 2 * NJ):
                qv[j, T:P0, :] = jnp.broadcast_to(qv[j, P0:P0 + 1, :], (HALO, 128))

        base = pl.multiple_of(t * T, T)
        attend(base, -T, T, pl.multiple_of(jnp.minimum(t, 0), T), True, CJ, CM,
               functools.partial(prepare_rows, t // 2, t % 2))
        quarter = pl.multiple_of(t * (T // 4), T // 4)
        project(quarter, base, wqv, 0, qv, 0)
        project(quarter, base, wqv, D // 4, qv, NJ)

    @_loop('O', NT)
    def _(t):
        zero = pl.multiple_of(jnp.minimum(t, 0), T)
        base = pl.multiple_of(t * T, T)
        gate = due(t < 0, list(norm(hs, base, 0, halves, hn, t * (T // 4), 0)), *OD)
        blocks = [jnp.concatenate([os[_ds(T + t * T + g * G + e * G // 2, G // 2), :] for g in range(T // G)], axis=0)
                  for e in range(2)]
        lhs = [a.astype(BF16) for a in _lhs_terms(*_even_odd(blocks[0]), *_even_odd(blocks[1]))]
        attend(pl.multiple_of(jnp.minimum(t * OP, T - OP), 16), S - T, OP, zero, False, CJW, CMW)
        for c in range(0, D // 2, NW):
            res = _strassen(lambda i: lhs[i], lambda i: _unpack(gate(wo[i, :, c:c + NW])))
            for r, half, val in _row_groups(res):
                cols = pl.ds(half * D // 2 + c, NW)
                hs[half * NJ // 2 + c // 128, _ds(base + (T + r), G // 2), :] = xs[_ds(base + r, G // 2), cols].astype(F32) + val

    list(norm(hs, S, 0, halves, hn, S // 4, 0))
    for c in cp_ffn:
        c.wait()

    @_loop('FFN', NT)
    def _(t):
        def matmul(lhs, w, c):
            k2, n2 = w.shape[0] // 2, w.shape[1] // 2

            def rhs(i):
                z = jnp.minimum(t, -CS[i]) + CS[i] if CS[i] >= 0 else 0
                return _rhs_terms(*(w[_ds(z + r, k2, 128), j + c:j + c + 128] for r in (0, k2) for j in (0, n2)))[i]
            return _strassen(lhs, lambda i: rhs(i).astype(BF16))

        lhs = normed(hn, (t + 1) * (T // 4))
        for c in range(0, F // 2, 128):
            gate, up = matmul(lhs, wg, c), matmul(lhs, wu, c)
            for i, term in enumerate(_lhs_terms(*map(_geglu, gate, up))):
                act[i, :, c:c + 128] = _pack(term)
        for c in range(0, D // 2, 128):
            for r, half, val in _row_groups(matmul(lambda i: _unpack(act[i]), wd, c)):
                cols = pl.ds(half * D // 2 + c, 128)
                xs[_ds(t * T + r, G // 2), cols] = (hs[half * NJ // 2 + c // 128, _ds(T + t * T + r, G // 2), :] + val).astype(BF16)
        cp_out(t).start()

    @_loop('drain', NT)
    def _(t):
        cp_out(t).wait()


@jax.jit
def pallas_sequential_preLN__sliding_local_dilated__glu_gated_geglu__prompt_kernel(
        A_x, A_wqkv, A_wo, B_x, B_w_gate, B_w_up, B_w_down):
    del B_x
    cfg = dict(CFG)
    flags = cfg.pop("FLAGS")
    any_spec = pl.BlockSpec(memory_space=pl.ANY)
    out = pl.pallas_call(
        functools.partial(_kernel, **cfg),
        in_specs=[any_spec] * 6,
        out_specs=any_spec,
        out_shape=jax.ShapeDtypeStruct((S, D), A_x.dtype),
        scratch_shapes=[
            pltpu.VMEM((S, D), BF16),
            pltpu.VMEM((3 * D, D), BF16),
            pltpu.VMEM((D, D), BF16),
            pltpu.VMEM((7, D // 4, D // 2), U32),
            pltpu.VMEM((7, D // 2, D // 2), U32),
            pltpu.VMEM((7, D // 4, D // 2), U32),
            pltpu.VMEM((D, F), BF16),
            pltpu.VMEM((D, F), BF16),
            pltpu.VMEM((F, D), BF16),
            pltpu.VMEM((H * ST, 128), U32),
            pltpu.VMEM((2, H * 9, 128), U32),
            pltpu.VMEM((7 * NJ // 2, (S + T) // 4, 128), U32),
            pltpu.VMEM((2 * NJ, P0 + S, 128), F32),
            pltpu.VMEM((NJ, P0 + S, 128), F32),
            pltpu.VMEM((W, T + 8, 128), F32),
            pltpu.VMEM((T + S, D), F32),
            pltpu.VMEM((NJ, T + S, 128), F32),
            pltpu.VMEM((7 * NJ // 2, (S + T) // 4, 128), U32),
            pltpu.VMEM((7, T // 4, F // 2), U32),
            pltpu.SemaphoreType.DMA((NT,)),
            pltpu.SemaphoreType.DMA((3 * NS,)),
            pltpu.SemaphoreType.DMA(()),
            pltpu.SemaphoreType.DMA((3,)),
            pltpu.SemaphoreType.DMA((NT,)),
        ],
        compiler_params=pltpu.CompilerParams(vmem_limit_bytes=120 * 1024 * 1024, flags=flags),
    )(A_x.reshape(S, D), A_wqkv, A_wo, B_w_gate, B_w_up, B_w_down)
    return out.reshape(A_x.shape)
```

```python
import functools
import math

import jax
import jax.numpy as jnp
from jax import lax
import jax.experimental.pallas as pl
import jax.experimental.pallas.tpu as pltpu

S, D, F = 2048, 1024, 3584
H, DH, W, DIL = 32, 32, 8, 2
T = 256
NT, NS, NJ = S // T, D // T, D // 128
HALO = 16
P0 = T + HALO
PITCH_C, PITCH_R = DH + 1, 9
G = 32
PIECE = 48
ORDER = (1, 3, 6, 4, 0, 2, 5)
SHARE = (0, None, 0, 1, None, 2, 1)
F32, BF16, U32 = jnp.float32, jnp.bfloat16, jnp.uint32


def _ln(x):
    m = jnp.mean(x, axis=-1, keepdims=True)
    c = x - m
    v = jnp.mean(c * c, axis=-1, keepdims=True)
    return c * lax.rsqrt(v + 1e-5)


def _geglu(g, u):
    c0 = math.sqrt(2.0 / math.pi)
    z = g * (c0 + (c0 * 0.044715) * (g * g))
    hg = 0.5 * g
    return (hg + hg * jnp.tanh(z)) * u


def _ds(start, size, align=None):
    if isinstance(start, int):
        return pl.ds(start, size)
    return pl.ds(pl.multiple_of(start, align or size), size)


def _tile(j):
    return slice(j * 128, (j + 1) * 128)


def _pack(x):
    return pltpu.bitcast(x.astype(BF16), U32)


def _unpack(x):
    return pltpu.bitcast(x, BF16)


def _lhs_terms(a11, a12, a21, a22):
    return a11 + a22, a21 + a22, a11, a22, a11 + a12, a21 - a11, a12 - a22


def _rhs_terms(b11, b12, b21, b22):
    f11, f12, f21, f22 = (b.astype(F32) for b in (b11, b12, b21, b22))
    return f11 + f22, b11, f12 - f22, f21 - f11, b22, f11 + f12, f21 + f22


def _strassen(lhs, rhs):
    m = {i: jnp.dot(lhs(i), rhs(i), preferred_element_type=F32) for i in ORDER}
    return m[3] + m[6] - m[4] + m[0], m[4] + m[2], m[1] + m[3], m[0] - m[1] + m[2] + m[5]


def _pieces(c, j):
    n = G // 2
    return [(i * G + q // 2 * n, q % 2 * NJ // 2 + j, c[q][i * n:(i + 1) * n])
            for q in range(4) for i in range(T // G)]


def _even_odd(y):
    return [jnp.concatenate([y[:, _tile(j)] for j in range(e, NJ, 2)], axis=1) for e in range(2)]


def _halves(y):
    return y[:, :D // 2], y[:, D // 2:]


def _due(never, tokens, first, last):
    count = [0]

    def gate(w):
        for i, token in enumerate(tokens):
            if first + i * (last - first) // (len(tokens) - 1) == count[0]:
                w = jnp.concatenate([jnp.where(never, token, w[:8]), w[8:]], axis=0)
        count[0] += 1
        return w
    return gate


def _kernel(x_hbm, wqkv_hbm, wo_hbm, wg_hbm, wu_hbm, wd_hbm, out_hbm,
            xs, raw, wk, wqv, wo, wg, wu, wd, tmp_c, tmp_r, xn, qv, ks, ps, att, hs, hn, act,
            sem_x, sem_w, sem_o, sem_f, sem_out):
    def cp_x(t):
        return pltpu.make_async_copy(x_hbm.at[_ds(t * T, T), :], xs.at[_ds(t * T, T), :], sem_x.at[t])

    def cp_w(u):
        col = (1, 0, 2)[u // NS] if isinstance(u, int) else jnp.where(u < NS, 1, u // NS * 2 - 2)
        return pltpu.make_async_copy(wqkv_hbm.at[_ds(u % NS * T, T), _ds(col * D, D)],
                                     raw.at[_ds(u * T, T), :], sem_w.at[u])

    cp_o = pltpu.make_async_copy(wo_hbm, raw.at[0:D, :], sem_o)
    cp_ffn = [pltpu.make_async_copy(src, dst, sem_f.at[i])
              for i, (src, dst) in enumerate(((wg_hbm, wg), (wu_hbm, wu), (wd_hbm, wd.at[:, 0:D])))]

    def cp_out(t, late):
        c, n = (D // 2 - 128, 128) if late else (0, D // 2 - 128)
        return [pltpu.make_async_copy(xs.at[_ds(t * T, T), j + c:j + c + n],
                                      out_hbm.at[_ds(t * T, T), j + c:j + c + n],
                                      sem_out.at[t * 4 + late * 2 + e]) for e, j in enumerate((0, D // 2))]

    def prepare_cols(u, dst, s):
        cols = pltpu.bitcast(raw[_ds(u * T, T), :], U32).T
        for h in range(H):
            tmp_c[h * PITCH_C:h * PITCH_C + DH, :] = cols[h * DH:(h + 1) * DH]

        def tile(j):
            rows = [tmp_c[pl.ds(4 * j + e, H, stride=PITCH_C), :] for e in range(4)]
            return _unpack(jnp.concatenate(rows, axis=0).T)

        tokens = []
        for j in range(NJ // 2):
            left, right = tile(j), tile(j + NJ // 2)
            terms = [_pack(b) for b in _rhs_terms(left[:128], right[:128], left[128:], right[128:])]
            for i, term in enumerate(terms):
                dst[i, _ds(s * 64, 64), _tile(j)] = term
            tokens.append(terms[-1][-8:])
        return tokens

    def prepare_rows(j, half, after):
        for e in range(2):
            for h in range(H):
                rows = raw[_ds(h * DH + half * (DH // 2), DH // 2), _ds((j + e * NJ // 2) * 128, 128)]
                tmp_r[e, h * PITCH_R:h * PITCH_R + 8, :] = pltpu.bitcast(rows, U32)
        for d in (0, 1, 2, 3, 8, 9, 10, 11):
            words = [tmp_r[e, pl.ds((d + k) // 2, H, stride=PITCH_R), :] for k in (0, 4) for e in range(2)]
            b11, b12, b21, b22 = (pltpu.bitcast(w >> 16 << 16 if d % 2 else w << 16, F32) for w in words)
            terms = _rhs_terms(after(b11), b12, b21, after(b22))
            for i, term in enumerate(terms):
                wo[i, _ds(half * 128 + (d // 8 * 4 + d % 8) * 16, 16), _ds(j * 128, 128)] = _pack(term)
            yield terms[-1]

    def norm(load, base, split, dst, dbase, doff):
        tokens = []
        for g in range(T // G):
            y = _ln(load(_ds(base + g * G, G)))
            terms = [_pack(a) for a in _lhs_terms(*split(y[:G // 2]), *split(y[G // 2:]))]
            for i, term in enumerate(terms):
                for j in range(NJ // 2):
                    dst[i * NJ // 2 + j, _ds(dbase + (doff + g * G // 4), G // 4), :] = term[:, _tile(j)]
            tokens.append(functools.reduce(jnp.bitwise_or, [terms[0][:, _tile(j)] for j in range(NJ // 2)]))
        return tokens

    def load_x(rows):
        return xs[rows, :].astype(F32)

    def load_h(rows):
        return jnp.concatenate([hs[j, rows, :] for j in range(NJ)], axis=1)

    def normed(src, row):
        return lambda i: _unpack(jnp.concatenate(
            [src[i * NJ // 2 + j, _ds(row, T // 4), :] for j in range(NJ // 2)], axis=1))

    def project(row, base, w, k0, out, plane, gate=lambda w: w):
        for j in range(NJ // 2):
            c = _strassen(normed(xn, row), lambda i: _unpack(gate(w[i, k0:k0 + D // 4, _tile(j)])))
            for r, col, val in _pieces(c, j):
                out[plane + col, _ds(base + (P0 + r), G // 2), :] = val

    def windows(ref, j, base, row, n):
        blk = [ref[j, pl.ds(base + (row - 8 - DIL * w), n + 8), :] for w in range(W // 2)]
        return [b[8:] for b in blk] + [b[:n] for b in blk]

    def attend(base, off, n, never, maybe_first, groups, side=None):
        token = []

        def after(x):
            return jnp.where(never, jnp.concatenate(token * (x.shape[0] // 8), axis=0), x) if token else x

        def mark(vals):
            token[:] = [functools.reduce(jnp.maximum, [v[i:i + 8] for v in vals for i in range(0, v.shape[0], 8)])]

        def dot(a, b):
            return functools.reduce(jnp.add, [x * y for x, y in zip(a, b)])

        def logits(r):
            q = [qv[j, _ds(base + (P0 + off + r), 8), :] for j in range(NJ)]
            k = [windows(ks, j, base, P0 + off + r, 8) for j in range(NJ)]
            ls = {}
            for group in groups:
                first = after(q[0])
                for w in group:
                    ls[w] = dot([first] + q[1:], [kj[w] for kj in k])
                mark([ls[w] for w in group])
            return [ls[w] for w in range(W)]

        def softmax(r, ls):
            ls = [l + pltpu.roll(l, 64, 1) for l in ls]
            ls = [l + pltpu.roll(l, 32, 1) for l in ls]
            if maybe_first and r < HALO:
                pos = base + (off + r) + lax.broadcasted_iota(jnp.int32, (8, 128), 0)
                ls = [jnp.where(pos >= DIL * w, l, -1e9 * DH ** 0.5) for w, l in enumerate(ls)]
            m = functools.reduce(jnp.maximum, ls)
            es = [jnp.exp2((l - m) * (DH ** -0.5 * math.log2(math.e))) for l in ls]
            inv = 1.0 / functools.reduce(jnp.add, es)
            for w in range(W):
                ps[w, r:r + 8, :] = es[w] * inv

        def mix(r):
            p = [ps[w, r:r + 16, :] for w in range(W)]
            for j in range(NJ):
                o = dot([after(p[0])] + p[1:], windows(qv, NJ + j, base, P0 + off + r, 16))
                att[_ds(base + (T + off + r), 16), _tile(j)] = o
                mark([o])

        side = side and side(after)
        pending = []
        for r in range(0, n + 32, 16):
            if side and r % 32 == 16 and r < n:
                mark([next(side)])
            new = [(r + i, logits(r + i)) for i in (0, 8)] if r < n else []
            if r >= 32:
                mix(r - 32)
            for job in pending:
                softmax(*job)
            pending = new

    def start_step(t):
        cp_x(t + 1).start()
        cp_w(NS + t).start()

    cp_w(0).start()
    cp_w(1).start()
    for ref, n in ((qv, P0), (ks, P0), (hs, T)):
        ref[:, 0:n, :] = jnp.zeros((ref.shape[0], n, 128), F32)

    @pl.loop(0, NS)
    def _(s):
        cp_w(s).wait()
        for i, start in enumerate((cp_w(2).start, cp_w(3).start, cp_x(0).start, lambda: start_step(0))):
            pl.when(s == i)(start)
        prepare_cols(s, wk, s)

    cp_x(0).wait()
    norm(load_x, 0, _even_odd, xn, 0, 0)
    start_step(1)

    @pl.loop(0, NT)
    def _(t):
        pl.when(t + 1 < NT)(lambda: cp_x(t + 1).wait())
        cp_w(NS + t).wait()
        pl.when(t + 3 < NT)(lambda: cp_x(t + 3).start())
        pl.when(t + 2 < NT)(lambda: cp_w(NS + t + 2).start())
        pl.when(t == NT - 2)(cp_o.start)
        row = pl.multiple_of(t * (T // 4), T // 4)
        jobs = (norm(load_x, jnp.minimum(t + 1, NT - 1) * T, _even_odd, xn, row, T // 4),
                prepare_cols(NS + t, wqv, t))
        tokens = [jobs[i].pop(0) for i in (0, 0, 0, 1, 0, 1, 0, 1, 0, 1, 0, 0)]
        project(row, t * T, wk, 0, ks, 0, _due(t < 0, tokens, 8, 27))

    cp_o.wait()
    for cp in cp_ffn:
        cp.start()

    @pl.loop(0, NT)
    def _(t):
        @pl.when(t == 1)
        def _():
            for j in range(NJ, 2 * NJ):
                qv[j, T:P0, :] = jnp.broadcast_to(qv[j, P0:P0 + 1, :], (HALO, 128))

        base = pl.multiple_of(t * T, T)
        attend(base, -T, T, t < 0, True, [(w,) for w in range(W)], functools.partial(prepare_rows, t // 2, t % 2))
        row = pl.multiple_of(t * (T // 4), T // 4)
        project(row, base, wqv, 0, qv, 0)
        project(row, base, wqv, D // 4, qv, NJ)

    @pl.loop(0, NT)
    def _(t):
        base = pl.multiple_of(t * T, T)
        gate = _due(t < 0, norm(load_h, base, _halves, hn, t * (T // 4), 0), 4, 20)
        blocks = [jnp.concatenate([att[_ds(T + t * T + g * G + e * G // 2, G // 2), :] for g in range(T // G)], axis=0)
                  for e in range(2)]
        lhs = [a.astype(BF16) for a in _lhs_terms(*_even_odd(blocks[0]), *_even_odd(blocks[1]))]
        piece = jnp.where(t == NT - 2, T - PIECE, jnp.minimum(t, NT - 3) * 32)
        attend(pl.multiple_of(piece, 16), S - T, PIECE, t < 0, False, [(w, w + W // 2) for w in range(W // 2)])
        for j in range(NJ // 2):
            c = _strassen(lambda i: lhs[i], lambda i: _unpack(gate(wo[i, :, _tile(j)])))
            for r, col, val in _pieces(c, j):
                hs[col, _ds(base + (T + r), G // 2), :] = xs[_ds(base + r, G // 2), _tile(col)].astype(F32) + val

    norm(load_h, S, _halves, hn, S // 4, 0)
    for cp in cp_ffn:
        cp.wait()

    @pl.loop(0, NT)
    def _(t):
        def matmul(lhs, w, k, n, j):
            def rhs(i):
                zero = 0 if SHARE[i] is None else jnp.minimum(t, -SHARE[i]) + SHARE[i]
                quads = (w[_ds(zero + r, k // 2, 128), _tile(c + j)] for r in (0, k // 2) for c in (0, n // 256))
                return _rhs_terms(*quads)[i].astype(BF16)
            return _strassen(lhs, rhs)

        lhs = normed(hn, (t + 1) * (T // 4))
        for j in range(F // 256):
            for i, term in enumerate(_lhs_terms(*map(_geglu, matmul(lhs, wg, D, F, j), matmul(lhs, wu, D, F, j)))):
                act[i, :, _tile(j)] = _pack(term)
        for j in range(NJ // 2):
            for r, col, val in _pieces(matmul(lambda i: _unpack(act[i]), wd, F, D, j), j):
                xs[_ds(t * T + r, G // 2), _tile(col)] = (hs[col, _ds(T + t * T + r, G // 2), :] + val).astype(BF16)
            if j >= NJ // 2 - 2:
                for cp in cp_out(t, j - (NJ // 2 - 2)):
                    cp.start()

    @pl.loop(0, NT)
    def _(t):
        for cp in cp_out(t, 0) + cp_out(t, 1):
            cp.wait()


@jax.jit
def pallas_sequential_preLN__sliding_local_dilated__glu_gated_geglu__prompt_kernel(
        A_x, A_wqkv, A_wo, B_x, B_w_gate, B_w_up, B_w_down):
    del B_x
    any_spec = pl.BlockSpec(memory_space=pl.ANY)
    out = pl.pallas_call(
        _kernel,
        in_specs=[any_spec] * 6,
        out_specs=any_spec,
        out_shape=jax.ShapeDtypeStruct((S, D), A_x.dtype),
        scratch_shapes=[
            pltpu.VMEM((S, D), BF16),
            pltpu.VMEM((3 * D, D), BF16),
            pltpu.VMEM((7, D // 4, D // 2), U32),
            pltpu.VMEM((7, D // 2, D // 2), U32),
            pltpu.VMEM((7, D // 4, D // 2), U32),
            pltpu.VMEM((D, F), BF16),
            pltpu.VMEM((D, F), BF16),
            pltpu.VMEM((F, D + 128), BF16),
            pltpu.VMEM((H * PITCH_C + 32, 128), U32),
            pltpu.VMEM((2, H * PITCH_R + 32, 128), U32),
            pltpu.VMEM((7 * NJ // 2, (S + T) // 4, 128), U32),
            pltpu.VMEM((2 * NJ, P0 + S, 128), F32),
            pltpu.VMEM((NJ, P0 + S, 128), F32),
            pltpu.VMEM((W, T, 128), F32),
            pltpu.VMEM((T + S, D), F32),
            pltpu.VMEM((NJ, T + S, 128), F32),
            pltpu.VMEM((7 * NJ // 2, (T + S) // 4, 128), U32),
            pltpu.VMEM((7, T // 4, F // 2), U32),
            pltpu.SemaphoreType.DMA((NT,)),
            pltpu.SemaphoreType.DMA((3 * NS,)),
            pltpu.SemaphoreType.DMA(()),
            pltpu.SemaphoreType.DMA((3,)),
            pltpu.SemaphoreType.DMA((4 * NT,)),
        ],
        compiler_params=pltpu.CompilerParams(vmem_limit_bytes=120 * 1024 * 1024),
    )(A_x.reshape(S, D), A_wqkv, A_wo, B_w_gate, B_w_up, B_w_down)
    return out.reshape(A_x.shape)
```

```python
import functools
import math

import jax
import jax.numpy as jnp
from jax import lax
import jax.experimental.pallas as pl
import jax.experimental.pallas.tpu as pltpu

S, D, F = 2048, 1024, 3584
H, DH, W, DIL = 32, 32, 8, 2
T = 256
NT, NS, NJ = S // T, D // T, D // 128
HALO = 16
P0 = T + HALO
PITCH_C, PITCH_R = DH + 1, 9
G = 32
PIECE = 48
ORDER = (1, 3, 6, 4, 0, 2, 5)
SHARE = (0, None, 0, 1, None, 2, 1)
F32, BF16, U32 = jnp.float32, jnp.bfloat16, jnp.uint32


def _ln(x):
    m = jnp.mean(x, axis=-1, keepdims=True)
    c = x - m
    v = jnp.mean(c * c, axis=-1, keepdims=True)
    return c * lax.rsqrt(v + 1e-5)


def _geglu(g, u):
    c0 = math.sqrt(2.0 / math.pi)
    z = g * (c0 + (c0 * 0.044715) * (g * g))
    hg = 0.5 * g
    return (hg + hg * jnp.tanh(z)) * u


def _ds(start, size, align=None):
    if isinstance(start, int):
        return pl.ds(start, size)
    return pl.ds(pl.multiple_of(start, align or size), size)


def _tile(j):
    return slice(j * 128, (j + 1) * 128)


def _pack(x):
    return pltpu.bitcast(x.astype(BF16), U32)


def _unpack(x):
    return pltpu.bitcast(x, BF16)


def _lhs_terms(a11, a12, a21, a22):
    return a11 + a22, a21 + a22, a11, a22, a11 + a12, a21 - a11, a12 - a22


def _rhs_terms(b11, b12, b21, b22):
    f11, f12, f21, f22 = (b.astype(F32) for b in (b11, b12, b21, b22))
    return f11 + f22, b11, f12 - f22, f21 - f11, b22, f11 + f12, f21 + f22


def _strassen(lhs, rhs):
    m = {i: jnp.dot(lhs(i), rhs(i), preferred_element_type=F32) for i in ORDER}
    return m[3] + m[6] - m[4] + m[0], m[4] + m[2], m[1] + m[3], m[0] - m[1] + m[2] + m[5]


def _pieces(c, j):
    n = G // 2
    return [(i * G + q // 2 * n, q % 2 * NJ // 2 + j, c[q][i * n:(i + 1) * n])
            for q in range(4) for i in range(T // G)]


def _even_odd(y):
    return [jnp.concatenate([y[:, _tile(j)] for j in range(e, NJ, 2)], axis=1) for e in range(2)]


def _halves(y):
    return y[:, :D // 2], y[:, D // 2:]


def _due(never, tokens, first, last):
    count = [0]

    def gate(w):
        for i, token in enumerate(tokens):
            if first + i * (last - first) // (len(tokens) - 1) == count[0]:
                w = jnp.concatenate([jnp.where(never, token, w[:8]), w[8:]], axis=0)
        count[0] += 1
        return w
    return gate


def _kernel(x_hbm, wqkv_hbm, wo_hbm, wg_hbm, wu_hbm, wd_hbm, out_hbm,
            xs, raw, wk, wqv, wo, wg, wu, wd, tmp_c, tmp_r, xn, qv, ks, ps, att, hs, hn, act,
            sem_x, sem_w, sem_o, sem_f, sem_out):
    def cp_x(t):
        return pltpu.make_async_copy(x_hbm.at[_ds(t * T, T), :], xs.at[_ds(t * T, T), :], sem_x.at[t])

    def cp_w(u):
        col = (1, 0, 2)[u // NS] if isinstance(u, int) else jnp.where(u < NS, 1, u // NS * 2 - 2)
        return pltpu.make_async_copy(wqkv_hbm.at[_ds(u % NS * T, T), _ds(col * D, D)],
                                     raw.at[_ds(u * T, T), :], sem_w.at[u])

    cp_o = pltpu.make_async_copy(wo_hbm, raw.at[0:D, :], sem_o)
    cp_ffn = [pltpu.make_async_copy(src, dst, sem_f.at[i])
              for i, (src, dst) in enumerate(((wg_hbm, wg), (wu_hbm, wu), (wd_hbm, wd.at[:, 0:D])))]

    def cp_out(t, late):
        c, n = (D // 2 - 128, 128) if late else (0, D // 2 - 128)
        return [pltpu.make_async_copy(xs.at[_ds(t * T, T), j + c:j + c + n],
                                      out_hbm.at[_ds(t * T, T), j + c:j + c + n],
                                      sem_out.at[t * 4 + late * 2 + e]) for e, j in enumerate((0, D // 2))]

    def prepare_cols(u, dst, s):
        cols = pltpu.bitcast(raw[_ds(u * T, T), :], U32).T
        for h in range(H):
            tmp_c[h * PITCH_C:h * PITCH_C + DH, :] = cols[h * DH:(h + 1) * DH]

        def tile(j):
            rows = [tmp_c[pl.ds(4 * j + e, H, stride=PITCH_C), :] for e in range(4)]
            return _unpack(jnp.concatenate(rows, axis=0).T)

        tokens = []
        for j in range(NJ // 2):
            left, right = tile(j), tile(j + NJ // 2)
            terms = [_pack(b) for b in _rhs_terms(left[:128], right[:128], left[128:], right[128:])]
            for i, term in enumerate(terms):
                dst[i, _ds(s * 64, 64), _tile(j)] = term
            tokens.append(terms[-1][-8:])
        return tokens

    def prepare_rows(j, half, after):
        for e in range(2):
            for h in range(H):
                rows = raw[_ds(h * DH + half * (DH // 2), DH // 2), _ds((j + e * NJ // 2) * 128, 128)]
                tmp_r[e, h * PITCH_R:h * PITCH_R + 8, :] = pltpu.bitcast(rows, U32)
        for d in (0, 1, 2, 3, 8, 9, 10, 11):
            words = [tmp_r[e, pl.ds((d + k) // 2, H, stride=PITCH_R), :] for k in (0, 4) for e in range(2)]
            b11, b12, b21, b22 = (pltpu.bitcast(w >> 16 << 16 if d % 2 else w << 16, F32) for w in words)
            terms = _rhs_terms(after(b11), b12, b21, after(b22))
            for i, term in enumerate(terms):
                wo[i, _ds(half * 128 + (d // 8 * 4 + d % 8) * 16, 16), _ds(j * 128, 128)] = _pack(term)
            yield terms[-1]

    def norm(load, base, split, dst, dbase, doff, n=T):
        tokens = []
        for g in range(n // G):
            y = _ln(load(_ds(base + g * G, G)))
            terms = [_pack(a) for a in _lhs_terms(*split(y[:G // 2]), *split(y[G // 2:]))]
            for i, term in enumerate(terms):
                for j in range(NJ // 2):
                    dst[i * NJ // 2 + j, _ds(dbase + (doff + g * G // 4), G // 4), :] = term[:, _tile(j)]
            tokens.append(functools.reduce(jnp.bitwise_or, [terms[0][:, _tile(j)] for j in range(NJ // 2)]))
        return tokens

    def load_x(rows):
        return xs[rows, :].astype(F32)

    def load_h(rows):
        return jnp.concatenate([hs[j, rows, :] for j in range(NJ)], axis=1)

    def normed(src, row):
        return lambda i: _unpack(jnp.concatenate(
            [src[i * NJ // 2 + j, _ds(row, T // 4), :] for j in range(NJ // 2)], axis=1))

    def project(row, base, w, k0, out, plane, gate=lambda w: w):
        for j in range(NJ // 2):
            c = _strassen(normed(xn, row), lambda i: _unpack(gate(w[i, k0:k0 + D // 4, _tile(j)])))
            for r, col, val in _pieces(c, j):
                out[plane + col, _ds(base + (P0 + r), G // 2), :] = val

    def windows(ref, j, base, row, n):
        blk = [ref[j, pl.ds(base + (row - 8 - DIL * w), n + 8), :] for w in range(W // 2)]
        return [b[8:] for b in blk] + [b[:n] for b in blk]

    def attend(base, off, n, never, maybe_first, groups, side=None):
        token = []

        def after(x):
            return jnp.where(never, jnp.concatenate(token * (x.shape[0] // 8), axis=0), x) if token else x

        def mark(vals):
            token[:] = [functools.reduce(jnp.maximum, [v[i:i + 8] for v in vals for i in range(0, v.shape[0], 8)])]

        def dot(a, b):
            return functools.reduce(jnp.add, [x * y for x, y in zip(a, b)])

        def logits(r):
            q = [qv[j, _ds(base + (P0 + off + r), 8), :] for j in range(NJ)]
            k = [windows(ks, j, base, P0 + off + r, 8) for j in range(NJ)]
            ls = {}
            for group in groups:
                first = after(q[0])
                for w in group:
                    ls[w] = dot([first] + q[1:], [kj[w] for kj in k])
                mark([ls[w] for w in group])
            return [ls[w] for w in range(W)]

        def softmax(r, ls):
            ls = [l + pltpu.roll(l, 64, 1) for l in ls]
            ls = [l + pltpu.roll(l, 32, 1) for l in ls]
            if maybe_first and r < HALO:
                pos = base + (off + r) + lax.broadcasted_iota(jnp.int32, (8, 128), 0)
                ls = [jnp.where(pos >= DIL * w, l, -1e9 * DH ** 0.5) for w, l in enumerate(ls)]
            m = functools.reduce(jnp.maximum, ls)
            es = [jnp.exp2((l - m) * (DH ** -0.5 * math.log2(math.e))) for l in ls]
            inv = 1.0 / functools.reduce(jnp.add, es)
            for w in range(W):
                ps[w, r:r + 8, :] = es[w] * inv
            return inv

        def mix(r):
            p = [ps[w, r:r + 16, :] for w in range(W)]
            for j in range(NJ):
                o = dot([after(p[0])] + p[1:], windows(qv, NJ + j, base, P0 + off + r, 16))
                att[_ds(base + (T + off + r), 16), _tile(j)] = o
                mark([o])

        side = side and side(after)
        pending = []
        for r in range(0, n + 32, 16):
            if side and r % 32 == 0 and r < n:
                mark([next(side)])
            new = [(r + i, logits(r + i)) for i in (0, 8)] if r < n else []
            if side and pending:
                mark(token + [softmax(*pending.pop(0))])
            if r >= 32:
                mix(r - 32)
            for job in pending:
                inv = softmax(*job)
                if side:
                    mark(token + [inv])
            pending = new

    def start_step(t):
        cp_x(t + 1).start()
        cp_w(NS + t).start()

    cp_w(0).start()
    cp_w(1).start()
    for ref, n in ((qv, P0), (ks, P0), (hs, T)):
        ref[:, 0:n, :] = jnp.zeros((ref.shape[0], n, 128), F32)

    @pl.loop(0, NS)
    def _(s):
        cp_w(s).wait()
        for i, start in enumerate((cp_w(2).start, cp_w(3).start, cp_x(0).start, lambda: start_step(0))):
            pl.when(s == i)(start)
        prepare_cols(s, wk, s)

    cp_x(0).wait()
    norm(load_x, 0, _even_odd, xn, 0, 0)
    start_step(1)

    @pl.loop(0, NT)
    def _(t):
        pl.when(t + 1 < NT)(lambda: cp_x(t + 1).wait())
        cp_w(NS + t).wait()
        pl.when(t + 3 < NT)(lambda: cp_x(t + 3).start())
        pl.when(t + 2 < NT)(lambda: cp_w(NS + t + 2).start())
        pl.when(t == NT - 2)(cp_o.start)
        row = pl.multiple_of(t * (T // 4), T // 4)
        jobs = (norm(load_x, jnp.minimum(t + 1, NT - 1) * T, _even_odd, xn, row, T // 4),
                prepare_cols(NS + t, wqv, t))
        tokens = [jobs[i].pop(0) for i in (0, 0, 0, 1, 0, 1, 0, 1, 0, 1, 0, 0)]
        project(row, t * T, wk, 0, ks, 0, _due(t < 0, tokens, 8, 27))

    cp_o.wait()
    for cp in cp_ffn:
        cp.start()

    @pl.loop(0, NT)
    def _(t):
        @pl.when(t == 1)
        def _():
            for j in range(NJ, 2 * NJ):
                qv[j, T:P0, :] = jnp.broadcast_to(qv[j, P0:P0 + 1, :], (HALO, 128))

        base = pl.multiple_of(t * T, T)
        attend(base, -T, T, t < 0, True, [(w,) for w in range(W)], functools.partial(prepare_rows, t // 2, t % 2))
        row = pl.multiple_of(t * (T // 4), T // 4)
        project(row, base, wqv, 0, qv, 0)
        project(row, base, wqv, D // 4, qv, NJ)

    @pl.loop(0, NT)
    def _(t):
        base = pl.multiple_of(t * T, T)
        gate = _due(t < 0, norm(load_h, base, _halves, hn, t * (T // 4), 0), 4, 20)
        blocks = [jnp.concatenate([att[_ds(T + t * T + g * G + e * G // 2, G // 2), :] for g in range(T // G)], axis=0)
                  for e in range(2)]
        lhs = [a.astype(BF16) for a in _lhs_terms(*_even_odd(blocks[0]), *_even_odd(blocks[1]))]
        piece = jnp.where(t == NT - 2, T - PIECE, jnp.minimum(t, NT - 3) * 32)
        attend(pl.multiple_of(piece, 16), S - T, PIECE, t < 0, False, [(w, w + W // 2) for w in range(W // 2)])
        for j in range(NJ // 2):
            c = _strassen(lambda i: lhs[i], lambda i: _unpack(gate(wo[i, :, _tile(j)])))
            for r, col, val in _pieces(c, j):
                hs[col, _ds(base + (T + r), G // 2), :] = xs[_ds(base + r, G // 2), _tile(col)].astype(F32) + val

    norm(load_h, S + T - G, _halves, hn, (S + T - G) // 4, 0, G)
    for cp in cp_ffn:
        cp.wait()

    @pl.loop(0, NT)
    def _(t):
        def matmul(lhs, w, k, n, j):
            def rhs(i):
                zero = 0 if SHARE[i] is None else jnp.minimum(t, -SHARE[i]) + SHARE[i]
                quads = (w[_ds(zero + r, k // 2, 128), _tile(c + j)] for r in (0, k // 2) for c in (0, n // 256))
                return _rhs_terms(*quads)[i].astype(BF16)
            return _strassen(lhs, rhs)

        lhs = normed(hn, (t + 1) * (T // 4))
        for j in range(F // 256):
            for i, term in enumerate(_lhs_terms(*map(_geglu, matmul(lhs, wg, D, F, j), matmul(lhs, wu, D, F, j)))):
                act[i, :, _tile(j)] = _pack(term)
        norm(load_h, S + t * G, _halves, hn, t * (G // 4), S // 4, G)
        for j in range(NJ // 2):
            for r, col, val in _pieces(matmul(lambda i: _unpack(act[i]), wd, F, D, j), j):
                xs[_ds(t * T + r, G // 2), _tile(col)] = (hs[col, _ds(T + t * T + r, G // 2), :] + val).astype(BF16)
            if j >= NJ // 2 - 2:
                for cp in cp_out(t, j - (NJ // 2 - 2)):
                    cp.start()

    @pl.loop(0, NT)
    def _(t):
        for cp in cp_out(t, 0) + cp_out(t, 1):
            cp.wait()


@jax.jit
def pallas_sequential_preLN__sliding_local_dilated__glu_gated_geglu__prompt_kernel(
        A_x, A_wqkv, A_wo, B_x, B_w_gate, B_w_up, B_w_down):
    del B_x
    any_spec = pl.BlockSpec(memory_space=pl.ANY)
    out = pl.pallas_call(
        _kernel,
        in_specs=[any_spec] * 6,
        out_specs=any_spec,
        out_shape=jax.ShapeDtypeStruct((S, D), A_x.dtype),
        scratch_shapes=[
            pltpu.VMEM((S, D), BF16),
            pltpu.VMEM((3 * D, D), BF16),
            pltpu.VMEM((7, D // 4, D // 2), U32),
            pltpu.VMEM((7, D // 2, D // 2), U32),
            pltpu.VMEM((7, D // 4, D // 2), U32),
            pltpu.VMEM((D, F), BF16),
            pltpu.VMEM((D, F), BF16),
            pltpu.VMEM((F, D + 128), BF16),
            pltpu.VMEM((H * PITCH_C + 32, 128), U32),
            pltpu.VMEM((2, H * PITCH_R + 32, 128), U32),
            pltpu.VMEM((7 * NJ // 2, (S + T) // 4, 128), U32),
            pltpu.VMEM((2 * NJ, P0 + S, 128), F32),
            pltpu.VMEM((NJ, P0 + S, 128), F32),
            pltpu.VMEM((W, T, 128), F32),
            pltpu.VMEM((T + S, D), F32),
            pltpu.VMEM((NJ, T + S, 128), F32),
            pltpu.VMEM((7 * NJ // 2, (T + S) // 4, 128), U32),
            pltpu.VMEM((7, T // 4, F // 2), U32),
            pltpu.SemaphoreType.DMA((NT,)),
            pltpu.SemaphoreType.DMA((3 * NS,)),
            pltpu.SemaphoreType.DMA(()),
            pltpu.SemaphoreType.DMA((3,)),
            pltpu.SemaphoreType.DMA((4 * NT,)),
        ],
        compiler_params=pltpu.CompilerParams(vmem_limit_bytes=120 * 1024 * 1024),
    )(A_x.reshape(S, D), A_wqkv, A_wo, B_w_gate, B_w_up, B_w_down)
    return out.reshape(A_x.shape)
```

```python
import functools
import math

import jax
import jax.numpy as jnp
from jax import lax
import jax.experimental.pallas as pl
import jax.experimental.pallas.tpu as pltpu

S, D, F = 2048, 1024, 3584
H, DH, W, DIL = 32, 32, 8, 2
T = 256
NT, NS, NJ = S // T, D // T, D // 128
HALO = 16
P0 = T + HALO
PITCH_C, PITCH_R = DH + 1, 9
G = 32
PIECE = 48
SLOPE = (-1.5, -0.5, 0.5, 1.5)
PAIRS = ((0, 1), (2, 3), (0, 2), (1, 3), (0, 3), (1, 2))
KEYS = ([(kind, i, i) for i in range(4) for kind in "pq"]
        + [key for i, j in PAIRS for key in (("v", i, j), ("z", i, j), ("v", j, i))])
F32, BF16, U32 = jnp.float32, jnp.bfloat16, jnp.uint32


def _ln(x):
    m = jnp.mean(x, axis=-1, keepdims=True)
    c = x - m
    v = jnp.mean(c * c, axis=-1, keepdims=True)
    return c * lax.rsqrt(v + 1e-5)


def _geglu(g, u):
    c0 = math.sqrt(2.0 / math.pi)
    z = g * (c0 + (c0 * 0.044715) * (g * g))
    hg = 0.5 * g
    return (hg + hg * jnp.tanh(z)) * u


def _ds(start, size, align=None):
    if isinstance(start, int):
        return pl.ds(start, size)
    return pl.ds(pl.multiple_of(start, align or size), size)


def _tile(j):
    return slice(j * 128, (j + 1) * 128)


def _pack(x):
    return pltpu.bitcast(x.astype(BF16), U32)


def _unpack(x):
    return pltpu.bitcast(x, BF16)


def _lhs_terms(a11, a12, a21, a22):
    return a11 + a22, a21 + a22, a11, a22, a11 + a12, a21 - a11, a12 - a22


def _rhs_terms(b11, b12, b21, b22):
    f11, f12, f21, f22 = (b.astype(F32) for b in (b11, b12, b21, b22))
    return f11 + f22, b11, f12 - f22, f21 - f11, b22, f11 + f12, f21 + f22


def _strassen(lhs, rhs):
    m = {i: jnp.dot(lhs(i), rhs(i), preferred_element_type=F32) for i in (1, 3, 6, 4, 0, 2, 5)}
    return m[3] + m[6] - m[4] + m[0], m[4] + m[2], m[1] + m[3], m[0] - m[1] + m[2] + m[5]


def _times(c, x):
    return x if c == 1 else c * x


def _lhs26(top, bot):
    y = [t * a + b for t, a, b in zip(SLOPE, top, bot)]
    out = {}
    for i in range(4):
        out["p", i, i], out["q", i, i] = top[i], y[i]
    for i, j in PAIRS:
        d, z = SLOPE[j] - SLOPE[i], y[i] - y[j]
        out["v", i, j], out["z", i, j], out["v", j, i] = _times(d, top[i]) + z, z, _times(d, top[j]) + z
    return [out[key] for key in KEYS]


def _rhs26(key, w):
    kind, i, j = key
    if kind == "v":
        return w(i, j)
    if kind == "z":
        return (w(j, i).astype(F32) - w(i, j).astype(F32)).astype(BF16)
    b = [(w(i, e) if kind == "p" else w(e, i)).astype(F32) for e in range(4)]
    return ((b[0] + b[1]) + (b[2] + b[3])).astype(BF16)


def _product26(lhs, rhs, pattern):
    pools = {c: iter([key for kind in kinds for key in KEYS if key[0] == kind])
             for c, kinds in (("d", "pq"), ("v", "v"), ("z", "z"))}
    top, bot, e, left = [None] * 4, [None] * 4, [None] * 6, [3] * 6

    def add(acc, i, x, negate=False):
        if acc[i] is None:
            acc[i] = (x, negate)
        elif acc[i][1] == negate:
            acc[i] = (acc[i][0] + x, negate)
        else:
            acc[i] = (acc[i][0] - x if negate else x - acc[i][0], False)

    for c in pattern:
        kind, i, j = key = next(pools[c])
        m = jnp.dot(lhs(KEYS.index(key)), rhs(key), preferred_element_type=F32)
        if kind == "p":
            add(top, i, m)
        if kind in "qv":
            add(bot, j, m, i > j)
        if kind in "vz":
            lo, hi = min(i, j), max(i, j)
            n = PAIRS.index((lo, hi))
            add(e, n, m, i > j)
            left[n] -= 1
            if not left[n]:
                x = _times(1.0 / (SLOPE[hi] - SLOPE[lo]), e[n][0])
                add(top, hi, x)
                add(top, lo, x, True)
    return [a for a, _ in top], [b - t * a for t, (a, _), (b, _) in zip(SLOPE, top, bot)]


def _pieces(blocks, cols):
    n = G // 2
    return [(g * G + q // len(cols) * n, cols[q % len(cols)], c[g * n:(g + 1) * n])
            for q, c in enumerate(blocks) for g in range(T // G)]


def _attn_terms(top, bot):
    return _lhs_terms(*(jnp.concatenate([y[:, _tile(j)] for j in range(e, NJ, 2)], axis=1)
                        for y in (top, bot) for e in range(2)))


def _ffn_terms(top, bot):
    return _lhs26(*([y[:, i * D // 4:(i + 1) * D // 4] for i in range(4)] for y in (top, bot)))


def _due(never, tokens, first, last):
    count = [0]

    def gate(w):
        for i, token in enumerate(tokens):
            if first + i * (last - first) // (len(tokens) - 1) == count[0]:
                w = jnp.concatenate([jnp.where(never, token, w[:8]), w[8:]], axis=0)
        count[0] += 1
        return w
    return gate


def _kernel(x_hbm, wqkv_hbm, wo_hbm, wg_hbm, wu_hbm, wd_hbm, out_hbm,
            xs, raw, wk, wqv, wo, wg, wu, wd, tmp_c, tmp_r, xn, qv, ks, ps, att, hs, act,
            sem_x, sem_w, sem_o, sem_f, sem_out):
    def cp_x(t):
        return pltpu.make_async_copy(x_hbm.at[_ds(t * T, T), :], xs.at[_ds(t * T, T), :], sem_x.at[t])

    def cp_w(u):
        col = (1, 0, 2)[u // NS] if isinstance(u, int) else jnp.where(u < NS, 1, u // NS * 2 - 2)
        return pltpu.make_async_copy(wqkv_hbm.at[_ds(u % NS * T, T), _ds(col * D, D)],
                                     raw.at[_ds(u * T, T), :], sem_w.at[u])

    cp_o = pltpu.make_async_copy(wo_hbm, raw.at[0:D, :], sem_o)
    cp_ffn = [pltpu.make_async_copy(src, dst, sem_f.at[i])
              for i, (src, dst) in enumerate(((wg_hbm, wg), (wu_hbm, wu), (wd_hbm, wd.at[:, 0:D])))]

    def cp_out(t, c):
        at = (_ds(t * T, T), pl.ds(c * D // 2, D // 2))
        return pltpu.make_async_copy(xs.at[at], out_hbm.at[at], sem_out.at[2 * t + c])

    def prepare_cols(u, dst, s):
        cols = pltpu.bitcast(raw[_ds(u * T, T), :], U32).T
        for h in range(H):
            tmp_c[h * PITCH_C:h * PITCH_C + DH, :] = cols[h * DH:(h + 1) * DH]

        def tile(j):
            rows = [tmp_c[pl.ds(4 * j + e, H, stride=PITCH_C), :] for e in range(4)]
            return _unpack(jnp.concatenate(rows, axis=0).T)

        tokens = []
        for j in range(NJ // 2):
            left, right = tile(j), tile(j + NJ // 2)
            terms = [_pack(b) for b in _rhs_terms(left[:128], right[:128], left[128:], right[128:])]
            for i, term in enumerate(terms):
                dst[i, _ds(s * 64, 64), _tile(j)] = term
            tokens.append(terms[-1][-8:])
        return tokens

    def prepare_rows(j, half, after):
        for e in range(2):
            for h in range(H):
                rows = raw[_ds(h * DH + half * (DH // 2), DH // 2), _ds((j + e * NJ // 2) * 128, 128)]
                tmp_r[e, h * PITCH_R:h * PITCH_R + 8, :] = pltpu.bitcast(rows, U32)
        for d in (0, 1, 2, 3, 8, 9, 10, 11):
            words = [tmp_r[e, pl.ds((d + k) // 2, H, stride=PITCH_R), :] for k in (0, 4) for e in range(2)]
            b11, b12, b21, b22 = (pltpu.bitcast(w >> 16 << 16 if d % 2 else w << 16, F32) for w in words)
            terms = _rhs_terms(after(b11), b12, b21, after(b22))
            for i, term in enumerate(terms):
                wo[i, _ds(half * 128 + (d // 8 * 4 + d % 8) * 16, 16), _ds(j * 128, 128)] = _pack(term)
            yield terms[-1]

    def norm(load, base, make_terms, dbase, doff, rows=T):
        tokens = []
        for g in range(rows // G):
            y = _ln(load(_ds(base + g * G, G)))
            terms = [_pack(a) for a in make_terms(y[:G // 2], y[G // 2:])]
            n = terms[0].shape[1] // 128
            for i, term in enumerate(terms):
                for j in range(n):
                    xn[i * n + j, _ds(dbase + (doff + g * G // 4), G // 4), :] = term[:, _tile(j)]
            last = terms[0 if make_terms is _attn_terms else -1]
            tokens.append(functools.reduce(jnp.bitwise_or, [last[:, _tile(j)] for j in range(n)]))
        return tokens

    def load_x(rows):
        return xs[rows, :].astype(F32)

    def load_h(rows):
        return jnp.concatenate([hs[j, rows, :] for j in range(NJ)], axis=1)

    def normed(row, n):
        return lambda i: _unpack(jnp.concatenate(
            [xn[i * n + j, _ds(row, T // 4), :] for j in range(n)], axis=1))

    def project(row, base, w, k0, out, plane, gate=lambda w: w):
        for j in range(NJ // 2):
            c = _strassen(normed(row, NJ // 2), lambda i: _unpack(gate(w[i, k0:k0 + D // 4, _tile(j)])))
            for r, col, val in _pieces(c, (j, j + NJ // 2)):
                out[plane + col, _ds(base + (P0 + r), G // 2), :] = val

    def windows(ref, j, base, row, n):
        blk = [ref[j, pl.ds(base + (row - 8 - DIL * w), n + 8), :] for w in range(W // 2)]
        return [b[8:] for b in blk] + [b[:n] for b in blk]

    def attend(base, off, n, never, maybe_first, groups, side=None):
        token = []

        def after(x):
            return jnp.where(never, jnp.concatenate(token * (x.shape[0] // 8), axis=0), x) if token else x

        def mark(vals):
            token[:] = [functools.reduce(jnp.maximum, [v[i:i + 8] for v in vals for i in range(0, v.shape[0], 8)])]

        def dot(a, b):
            return functools.reduce(jnp.add, [x * y for x, y in zip(a, b)])

        def logits(r):
            q = [qv[j, _ds(base + (P0 + off + r), 8), :] for j in range(NJ)]
            k = [windows(ks, j, base, P0 + off + r, 8) for j in range(NJ)]
            ls = {}
            for group in groups:
                first = after(q[0])
                for w in group:
                    ls[w] = dot([first] + q[1:], [kj[w] for kj in k])
                mark([ls[w] for w in group])
            return [ls[w] for w in range(W)]

        def softmax(r, ls):
            ls = [l + pltpu.roll(l, 64, 1) for l in ls]
            ls = [l + pltpu.roll(l, 32, 1) for l in ls]
            if maybe_first and r < HALO:
                pos = base + (off + r) + lax.broadcasted_iota(jnp.int32, (8, 128), 0)
                ls = [jnp.where(pos >= DIL * w, l, -1e9 * DH ** 0.5) for w, l in enumerate(ls)]
            m = functools.reduce(jnp.maximum, ls)
            es = [jnp.exp2((l - m) * (DH ** -0.5 * math.log2(math.e))) for l in ls]
            inv = 1.0 / functools.reduce(jnp.add, es)
            for w in range(W):
                ps[w, r:r + 8, :] = es[w] * inv
            return inv

        def mix(r):
            p = [ps[w, r:r + 16, :] for w in range(W)]
            for j in range(NJ):
                o = dot([after(p[0])] + p[1:], windows(qv, NJ + j, base, P0 + off + r, 16))
                att[_ds(base + (T + off + r), 16), _tile(j)] = o
                mark([o])

        side = side and side(after)
        pending = []
        for r in range(0, n + 32, 16):
            if side and r % 32 == 0 and r < n:
                mark([next(side)])
            new = [(r + i, logits(r + i)) for i in (0, 8)] if r < n else []
            if side and pending:
                mark(token + [softmax(*pending.pop(0))])
            if r >= 32:
                mix(r - 32)
            for job in pending:
                inv = softmax(*job)
                if side:
                    mark(token + [inv])
            pending = new

    def start_step(t):
        cp_x(t + 1).start()
        cp_w(NS + t).start()

    cp_w(0).start()
    cp_w(1).start()
    for ref, n in ((qv, P0), (ks, P0), (hs, T)):
        ref[:, 0:n, :] = jnp.zeros((ref.shape[0], n, 128), F32)

    @pl.loop(0, NS)
    def _(s):
        cp_w(s).wait()
        for i, start in enumerate((cp_w(2).start, cp_w(3).start, cp_x(0).start, lambda: start_step(0))):
            pl.when(s == i)(start)
        prepare_cols(s, wk, s)

    cp_x(0).wait()
    norm(load_x, 0, _attn_terms, 0, 0)
    start_step(1)

    @pl.loop(0, NT)
    def _(t):
        pl.when(t + 1 < NT)(lambda: cp_x(t + 1).wait())
        cp_w(NS + t).wait()
        pl.when(t + 3 < NT)(lambda: cp_x(t + 3).start())
        pl.when(t + 2 < NT)(lambda: cp_w(NS + t + 2).start())
        pl.when(t == NT - 2)(cp_o.start)
        row = pl.multiple_of(t * (T // 4), T // 4)
        jobs = (norm(load_x, jnp.minimum(t + 1, NT - 1) * T, _attn_terms, row, T // 4),
                prepare_cols(NS + t, wqv, t))
        tokens = [jobs[i].pop(0) for i in (0, 0, 0, 1, 0, 1, 0, 1, 0, 1, 0, 0)]
        project(row, t * T, wk, 0, ks, 0, _due(t < 0, tokens, 8, 27))

    cp_o.wait()
    for cp in cp_ffn:
        cp.start()

    @pl.loop(0, NT)
    def _(t):
        @pl.when(t == 1)
        def _():
            for j in range(NJ, 2 * NJ):
                qv[j, T:P0, :] = jnp.broadcast_to(qv[j, P0:P0 + 1, :], (HALO, 128))

        base = pl.multiple_of(t * T, T)
        attend(base, -T, T, t < 0, True, [(w,) for w in range(W)], functools.partial(prepare_rows, t // 2, t % 2))
        row = pl.multiple_of(t * (T // 4), T // 4)
        project(row, base, wqv, 0, qv, 0)
        project(row, base, wqv, D // 4, qv, NJ)

    @pl.loop(0, NT)
    def _(t):
        base = pl.multiple_of(t * T, T)
        gate = _due(t < 0, norm(load_h, base, _ffn_terms, t * (T // 4), 0), 3, 27)
        blocks = [jnp.concatenate([att[_ds(T + t * T + g * G + e * G // 2, G // 2), :] for g in range(T // G)], axis=0)
                  for e in range(2)]
        lhs = [a.astype(BF16) for a in _attn_terms(*blocks)]
        piece = jnp.where(t == NT - 2, T - PIECE, jnp.minimum(t, NT - 3) * 32)
        attend(pl.multiple_of(piece, 16), S - T, PIECE, t < 0, False, [(w, w + W // 2) for w in range(W // 2)])
        for j in range(NJ // 2):
            c = _strassen(lambda i: lhs[i], lambda i: _unpack(gate(wo[i, :, _tile(j)])))
            for r, col, val in _pieces(c, (j, j + NJ // 2)):
                hs[col, _ds(base + (T + r), G // 2), :] = xs[_ds(base + r, G // 2), _tile(col)].astype(F32) + val

    norm(load_h, S + T - G, _ffn_terms, (S + T - G) // 4, 0, G)
    for cp in cp_ffn:
        cp.wait()

    @pl.loop(0, NT)
    def _(t):
        def matmul(lhs, w, cols, pattern):
            def rhs(key):
                n, k = "v zpq".index(key[0]), w.shape[0] // 4
                zero = jnp.minimum(t, -n) + n if n else 0
                return _rhs26(key, lambda i, j: w[_ds(zero + i * k, k, 128), _tile(cols[j])])
            return _product26(lhs, rhs, pattern)

        lhs = normed((t + 1) * (T // 4), NJ // 4)
        for c in range(F // 512):
            gate, up = (matmul(lhs, w, range(c, F // 128, F // 512), "vdvzvdvzdvdvzvdvzdvdvzvdvz") for w in (wg, wu))
            for i, term in enumerate(_lhs26(*(list(map(_geglu, g, u)) for g, u in zip(gate, up)))):
                act[i, :, _tile(c)] = _pack(term)
        norm(load_h, S + t * G, _ffn_terms, t * (G // 4), S // 4, G)
        for c in range(2):
            cols = range(4 * c, 4 * c + 4)
            top, bot = matmul(lambda i: _unpack(act[i]), wd, cols, "vzvvzvdvzdvdvzdvdvzdvdvzdv")
            for r, col, val in _pieces(top + bot, cols):
                xs[_ds(t * T + r, G // 2), _tile(col)] = (hs[col, _ds(T + t * T + r, G // 2), :] + val).astype(BF16)
            cp_out(t, c).start()

    @pl.loop(0, NT)
    def _(t):
        cp_out(t, 0).wait()
        cp_out(t, 1).wait()


@jax.jit
def pallas_sequential_preLN__sliding_local_dilated__glu_gated_geglu__prompt_kernel(
        A_x, A_wqkv, A_wo, B_x, B_w_gate, B_w_up, B_w_down):
    del B_x
    any_spec = pl.BlockSpec(memory_space=pl.ANY)
    out = pl.pallas_call(
        _kernel,
        in_specs=[any_spec] * 6,
        out_specs=any_spec,
        out_shape=jax.ShapeDtypeStruct((S, D), A_x.dtype),
        scratch_shapes=[
            pltpu.VMEM((S, D), BF16),
            pltpu.VMEM((3 * D, D), BF16),
            pltpu.VMEM((7, D // 4, D // 2), U32),
            pltpu.VMEM((7, D // 2, D // 2), U32),
            pltpu.VMEM((7, D // 4, D // 2), U32),
            pltpu.VMEM((D, F), BF16),
            pltpu.VMEM((D, F), BF16),
            pltpu.VMEM((F, D + 128), BF16),
            pltpu.VMEM((H * PITCH_C + 32, 128), U32),
            pltpu.VMEM((2, H * PITCH_R + 32, 128), U32),
            pltpu.VMEM((26 * NJ // 4, (S + T) // 4, 128), U32),
            pltpu.VMEM((2 * NJ, P0 + S, 128), F32),
            pltpu.VMEM((NJ, P0 + S, 128), F32),
            pltpu.VMEM((W, T, 128), F32),
            pltpu.VMEM((T + S, D), F32),
            pltpu.VMEM((NJ, T + S, 128), F32),
            pltpu.VMEM((26, T // 4, F // 4), U32),
            pltpu.SemaphoreType.DMA((NT,)),
            pltpu.SemaphoreType.DMA((3 * NS,)),
            pltpu.SemaphoreType.DMA(()),
            pltpu.SemaphoreType.DMA((3,)),
            pltpu.SemaphoreType.DMA((2 * NT,)),
        ],
        compiler_params=pltpu.CompilerParams(vmem_limit_bytes=120 * 1024 * 1024),
    )(A_x.reshape(S, D), A_wqkv, A_wo, B_w_gate, B_w_up, B_w_down)
    return out.reshape(A_x.shape)
```

```python
import functools
import math

import jax
import jax.numpy as jnp
from jax import lax
import jax.experimental.pallas as pl
import jax.experimental.pallas.tpu as pltpu

S, D, F = 2048, 1024, 3584
H, DH, W, DIL = 32, 32, 8, 2
T = 256
NT, NS, NJ = S // T, D // T, D // 128
HALO = 16
P0 = T + HALO
PITCH_C, PITCH_R = DH + 1, 9
G = 32
PIECE = 48
SLOPE = (-1.5, -0.5, 0.5, 1.5)
PAIRS = ((0, 1), (2, 3), (0, 2), (1, 3), (0, 3), (1, 2))
KEYS = ([(kind, i, i) for i in range(4) for kind in "pq"]
        + [key for i, j in PAIRS for key in (("v", i, j), ("z", i, j), ("v", j, i))])
F32, BF16, U32 = jnp.float32, jnp.bfloat16, jnp.uint32


def _ln(x):
    m = jnp.mean(x, axis=-1, keepdims=True)
    c = x - m
    v = jnp.mean(c * c, axis=-1, keepdims=True)
    return c * lax.rsqrt(v + 1e-5)


def _geglu2(g, u):
    c0 = math.sqrt(2.0 / math.pi)
    z = g * (c0 + (c0 * 0.044715) * (g * g))
    return (g + g * jnp.tanh(z)) * u


def _ds(start, size, align=None):
    if isinstance(start, int):
        return pl.ds(start, size)
    return pl.ds(pl.multiple_of(start, align or size), size)


def _tile(j):
    return slice(j * 128, (j + 1) * 128)


def _pack(x):
    return pltpu.bitcast(x.astype(BF16), U32)


def _unpack(x):
    return pltpu.bitcast(x, BF16)


def _lhs_terms(a11, a12, a21, a22):
    return a11 + a22, a21 + a22, a11, a22, a11 + a12, a21 - a11, a12 - a22


def _rhs_terms(b11, b12, b21, b22):
    f11, f12, f21, f22 = (b.astype(F32) for b in (b11, b12, b21, b22))
    return f11 + f22, b11, f12 - f22, f21 - f11, b22, f11 + f12, f21 + f22


def _strassen(lhs, rhs):
    m = {i: jnp.dot(lhs(i), rhs(i), preferred_element_type=F32) for i in (1, 3, 6, 4, 0, 2, 5)}
    return m[3] + m[6] - m[4] + m[0], m[4] + m[2], m[1] + m[3], m[0] - m[1] + m[2] + m[5]


def _times(c, x):
    return x if c == 1 else c * x


def _lhs26(top, bot):
    y = [t * a + b for t, a, b in zip(SLOPE, top, bot)]
    out = {}
    for i in range(4):
        out["p", i, i], out["q", i, i] = top[i], y[i]
    for i, j in PAIRS:
        d, z = SLOPE[j] - SLOPE[i], y[i] - y[j]
        out["v", i, j], out["z", i, j], out["v", j, i] = _times(d, top[i]) + z, z, _times(d, top[j]) + z
    return [out[key] for key in KEYS]


def _rhs26(key, w):
    kind, i, j = key
    if kind == "v":
        return w(i, j)
    if kind == "z":
        return (w(j, i).astype(F32) - w(i, j).astype(F32)).astype(BF16)
    b = [(w(i, e) if kind == "p" else w(e, i)).astype(F32) for e in range(4)]
    return ((b[0] + b[1]) + (b[2] + b[3])).astype(BF16)


def _product26(lhs, rhs, pattern):
    pools = {c: iter([key for kind in kinds for key in KEYS if key[0] == kind])
             for c, kinds in (("d", "pq"), ("v", "v"), ("z", "z"))}
    top, bot, e, left = [None] * 4, [None] * 4, [None] * 6, [3] * 6

    def add(acc, i, x, negate=False):
        if acc[i] is None:
            acc[i] = (x, negate)
        elif acc[i][1] == negate:
            acc[i] = (acc[i][0] + x, negate)
        else:
            acc[i] = (acc[i][0] - x if negate else x - acc[i][0], False)

    for c in pattern:
        kind, i, j = key = next(pools[c])
        m = jnp.dot(lhs(KEYS.index(key)), rhs(key), preferred_element_type=F32)
        if kind == "p":
            add(top, i, m)
        if kind in "qv":
            add(bot, j, m, i > j)
        if kind in "vz":
            lo, hi = min(i, j), max(i, j)
            n = PAIRS.index((lo, hi))
            add(e, n, m, i > j)
            left[n] -= 1
            if not left[n]:
                x = _times(1.0 / (SLOPE[hi] - SLOPE[lo]), e[n][0])
                add(top, hi, x)
                add(top, lo, x, True)
    return [a for a, _ in top], [b - t * a for t, (a, _), (b, _) in zip(SLOPE, top, bot)]


def _pieces(blocks, cols):
    n = G // 2
    return [(g * G + q // len(cols) * n, cols[q % len(cols)], c[g * n:(g + 1) * n])
            for q, c in enumerate(blocks) for g in range(T // G)]


def _attn_terms(top, bot):
    return _lhs_terms(*(jnp.concatenate([y[:, _tile(j)] for j in range(e, NJ, 2)], axis=1)
                        for y in (top, bot) for e in range(2)))


def _ffn_terms(top, bot):
    return _lhs26(*([y[:, i * D // 4:(i + 1) * D // 4] for i in range(4)] for y in (top, bot)))


def _due(never, tokens, first, last):
    count = [0]

    def gate(w):
        for i, token in enumerate(tokens):
            if first + i * (last - first) // (len(tokens) - 1) == count[0]:
                w = jnp.concatenate([jnp.where(never, token, w[:8]), w[8:]], axis=0)
        count[0] += 1
        return w
    return gate


def _kernel(x_hbm, wqkv_hbm, wo_hbm, wg_hbm, wu_hbm, wd_hbm, out_hbm,
            xs, raw, wk, wqv, wo, wg, wu, wd, tmp_c, tmp_r, xn, qv, ks, ps, att, hs, act,
            sem_x, sem_w, sem_o, sem_f, sem_out):
    def cp_x(t):
        return pltpu.make_async_copy(x_hbm.at[_ds(t * T, T), :], xs.at[_ds(t * T, T), :], sem_x.at[t])

    def cp_w(u):
        col = (1, 0, 2)[u // NS] if isinstance(u, int) else jnp.where(u < NS, 1, u // NS * 2 - 2)
        return pltpu.make_async_copy(wqkv_hbm.at[_ds(u % NS * T, T), _ds(col * D, D)],
                                     raw.at[_ds(u * T, T), :], sem_w.at[u])

    cp_o = pltpu.make_async_copy(wo_hbm, raw.at[0:D, :], sem_o)
    cp_ffn = [pltpu.make_async_copy(src, dst, sem_f.at[i])
              for i, (src, dst) in enumerate(((wg_hbm, wg), (wu_hbm, wu), (wd_hbm, wd.at[:, 0:D])))]

    def cp_out(t, c):
        at = (_ds(t * T, T), pl.ds(c * D // 2, D // 2))
        return pltpu.make_async_copy(xs.at[at], out_hbm.at[at], sem_out.at[2 * t + c])

    def prepare_cols(u, dst, s):
        cols = pltpu.bitcast(raw[_ds(u * T, T), :], U32).T
        for h in range(H):
            tmp_c[h * PITCH_C:h * PITCH_C + DH, :] = cols[h * DH:(h + 1) * DH]

        def tile(j):
            rows = [tmp_c[pl.ds(4 * j + e, H, stride=PITCH_C), :] for e in range(4)]
            return _unpack(jnp.concatenate(rows, axis=0).T)

        tokens = []
        for j in range(NJ // 2):
            left, right = tile(j), tile(j + NJ // 2)
            terms = [_pack(b) for b in _rhs_terms(left[:128], right[:128], left[128:], right[128:])]
            for i, term in enumerate(terms):
                dst[i, _ds(s * 64, 64), _tile(j)] = term
            tokens.append(terms[-1][-8:])
        return tokens

    def prepare_rows(j, half, after):
        for e in range(2):
            for h in range(H):
                rows = raw[_ds(h * DH + half * (DH // 2), DH // 2), _ds((j + e * NJ // 2) * 128, 128)]
                tmp_r[e, h * PITCH_R:h * PITCH_R + 8, :] = pltpu.bitcast(rows, U32)
        for d in (0, 1, 2, 3, 8, 9, 10, 11):
            words = [tmp_r[e, pl.ds((d + k) // 2, H, stride=PITCH_R), :] for k in (0, 4) for e in range(2)]
            b11, b12, b21, b22 = (pltpu.bitcast(w >> 16 << 16 if d % 2 else w << 16, F32) for w in words)
            terms = _rhs_terms(after(b11), b12, b21, after(b22))
            for i, term in enumerate(terms):
                wo[i, _ds(half * 128 + (d // 8 * 4 + d % 8) * 16, 16), _ds(j * 128, 128)] = _pack(term)
            yield terms[-1]

    def norm(load, base, make_terms, dbase, doff, rows=T):
        tokens = []
        for g in range(rows // G):
            y = _ln(load(_ds(base + g * G, G)))
            terms = [_pack(a) for a in make_terms(y[:G // 2], y[G // 2:])]
            n = terms[0].shape[1] // 128
            for i, term in enumerate(terms):
                for j in range(n):
                    xn[i * n + j, _ds(dbase + (doff + g * G // 4), G // 4), :] = term[:, _tile(j)]
            last = terms[0 if make_terms is _attn_terms else -1]
            tokens.append(functools.reduce(jnp.bitwise_or, [last[:, _tile(j)] for j in range(n)]))
        return tokens

    def load_x(rows):
        return xs[rows, :].astype(F32)

    def load_h(rows):
        return jnp.concatenate([hs[j, rows, :] for j in range(NJ)], axis=1)

    def normed(row, n):
        return lambda i: _unpack(jnp.concatenate(
            [xn[i * n + j, _ds(row, T // 4), :] for j in range(n)], axis=1))

    def project(row, base, w, k0, out, plane, gate=lambda w: w):
        for j in range(NJ // 2):
            c = _strassen(normed(row, NJ // 2), lambda i: _unpack(gate(w[i, k0:k0 + D // 4, _tile(j)])))
            for r, col, val in _pieces(c, (j, j + NJ // 2)):
                out[plane + col, _ds(base + (P0 + r), G // 2), :] = val

    def windows(ref, j, base, row, n):
        blk = [ref[j, pl.ds(base + (row - 8 - DIL * w), n + 8), :] for w in range(W // 2)]
        return [b[8:] for b in blk] + [b[:n] for b in blk]

    def attend(base, off, n, never, maybe_first, groups, side=None):
        token = []

        def after(x):
            return jnp.where(never, jnp.concatenate(token * (x.shape[0] // 8), axis=0), x) if token else x

        def mark(vals):
            token[:] = [functools.reduce(jnp.maximum, [v[i:i + 8] for v in vals for i in range(0, v.shape[0], 8)])]

        def dot(a, b):
            return functools.reduce(jnp.add, [x * y for x, y in zip(a, b)])

        def logits(r):
            q = [qv[j, _ds(base + (P0 + off + r), 8), :] for j in range(NJ)]
            k = [windows(ks, j, base, P0 + off + r, 8) for j in range(NJ)]
            ls = {}
            for group in groups:
                first = after(q[0])
                for w in group:
                    ls[w] = dot([first] + q[1:], [kj[w] for kj in k])
                mark([ls[w] for w in group])
            return [ls[w] for w in range(W)]

        def softmax(r, ls):
            ls = [l + pltpu.roll(l, 64, 1) for l in ls]
            ls = [l + pltpu.roll(l, 32, 1) for l in ls]
            if maybe_first and r < HALO:
                pos = base + (off + r) + lax.broadcasted_iota(jnp.int32, (8, 128), 0)
                ls = [jnp.where(pos >= DIL * w, l, -1e9 * DH ** 0.5) for w, l in enumerate(ls)]
            m = functools.reduce(jnp.maximum, ls)
            es = [jnp.exp2((l - m) * (DH ** -0.5 * math.log2(math.e))) for l in ls]
            inv = 1.0 / functools.reduce(jnp.add, es)
            for w in range(W):
                ps[w, r:r + 8, :] = es[w] * inv
            return inv

        def mix(r):
            p = [ps[w, r:r + 16, :] for w in range(W)]
            for j in range(NJ):
                o = dot([after(p[0])] + p[1:], windows(qv, NJ + j, base, P0 + off + r, 16))
                att[_ds(base + (T + off + r), 16), _tile(j)] = o
                mark([o])

        side = side and side(after)
        pending = []
        for r in range(0, n + 32, 16):
            if side and r % 32 == 0 and r < n:
                mark([next(side)])
            new = [(r + i, logits(r + i)) for i in (0, 8)] if r < n else []
            if side and pending:
                mark(token + [softmax(*pending.pop(0))])
            if r >= 32:
                mix(r - 32)
            for job in pending:
                inv = softmax(*job)
                if side:
                    mark(token + [inv])
            pending = new

    def start_step(t):
        cp_x(t + 1).start()
        cp_w(NS + t).start()

    cp_w(0).start()
    cp_w(1).start()
    for ref, n in ((qv, P0), (ks, P0), (hs, T)):
        ref[:, 0:n, :] = jnp.zeros((ref.shape[0], n, 128), F32)

    @pl.loop(0, NS)
    def _(s):
        cp_w(s).wait()
        for i, start in enumerate((cp_w(2).start, cp_w(3).start, cp_x(0).start, lambda: start_step(0))):
            pl.when(s == i)(start)
        prepare_cols(s, wk, s)

    cp_x(0).wait()
    norm(load_x, 0, _attn_terms, 0, 0)
    start_step(1)

    @pl.loop(0, NT)
    def _(t):
        pl.when(t + 1 < NT)(lambda: cp_x(t + 1).wait())
        cp_w(NS + t).wait()
        pl.when(t + 3 < NT)(lambda: cp_x(t + 3).start())
        pl.when(t + 2 < NT)(lambda: cp_w(NS + t + 2).start())
        pl.when(t == NT - 2)(cp_o.start)
        row = pl.multiple_of(t * (T // 4), T // 4)
        jobs = (norm(load_x, jnp.minimum(t + 1, NT - 1) * T, _attn_terms, row, T // 4),
                prepare_cols(NS + t, wqv, t))
        tokens = [jobs[i].pop(0) for i in (0, 0, 0, 1, 0, 1, 0, 1, 0, 1, 0, 0)]
        project(row, t * T, wk, 0, ks, 0, _due(t < 0, tokens, 8, 27))

    cp_o.wait()
    for cp in cp_ffn:
        cp.start()

    @pl.loop(0, NT)
    def _(t):
        @pl.when(t == 1)
        def _():
            for j in range(NJ, 2 * NJ):
                qv[j, T:P0, :] = jnp.broadcast_to(qv[j, P0:P0 + 1, :], (HALO, 128))

        base = pl.multiple_of(t * T, T)
        attend(base, -T, T, t < 0, True, [(w,) for w in range(W)], functools.partial(prepare_rows, t // 2, t % 2))
        row = pl.multiple_of(t * (T // 4), T // 4)
        project(row, base, wqv, 0, qv, 0)
        project(row, base, wqv, D // 4, qv, NJ)

    @pl.loop(0, NT)
    def _(t):
        base = pl.multiple_of(t * T, T)
        gate = _due(t < 0, norm(load_h, base, _ffn_terms, t * (T // 4), 0), 3, 27)
        blocks = [jnp.concatenate([att[_ds(T + t * T + g * G + e * G // 2, G // 2), :] for g in range(T // G)], axis=0)
                  for e in range(2)]
        lhs = [a.astype(BF16) for a in _attn_terms(*blocks)]
        piece = jnp.where(t == NT - 2, T - PIECE, jnp.minimum(t, NT - 3) * 32)
        attend(pl.multiple_of(piece, 16), S - T, PIECE, t < 0, False, [(w, w + W // 2) for w in range(W // 2)])
        for j in range(NJ // 2):
            c = _strassen(lambda i: lhs[i], lambda i: _unpack(gate(wo[i, :, _tile(j)])))
            for r, col, val in _pieces(c, (j, j + NJ // 2)):
                hs[col, _ds(base + (T + r), G // 2), :] = xs[_ds(base + r, G // 2), _tile(col)].astype(F32) + val

    norm(load_h, S + T - G, _ffn_terms, (S + T - G) // 4, 0, G)
    for cp in cp_ffn:
        cp.wait()

    @pl.loop(0, NT)
    def _(t):
        def matmul(lhs, w, cols, pattern):
            def rhs(key):
                n, k = "v zpq".index(key[0]), w.shape[0] // 4
                zero = jnp.minimum(t, -n) + n if n else 0
                return _rhs26(key, lambda i, j: w[_ds(zero + i * k, k, 128), _tile(cols[j])])
            return _product26(lhs, rhs, pattern)

        lhs = normed((t + 1) * (T // 4), NJ // 4)
        for c in range(F // 512):
            gate, up = (matmul(lhs, w, range(c, F // 128, F // 512), "vdvzvdvzdvdvzvdvzdvdvzvdvz") for w in (wg, wu))
            for i, term in enumerate(_lhs26(*(list(map(_geglu2, g, u)) for g, u in zip(gate, up)))):
                act[i, :, _tile(c)] = _pack(term)
        norm(load_h, S + t * G, _ffn_terms, t * (G // 4), S // 4, G)
        for c in range(2):
            cols = range(4 * c, 4 * c + 4)
            top, bot = matmul(lambda i: _unpack(act[i]), wd, cols, "vzvvzvdvzdvdvzdvdvzdvdvzdv")
            for r, col, val in _pieces(top + bot, cols):
                xs[_ds(t * T + r, G // 2), _tile(col)] = (hs[col, _ds(T + t * T + r, G // 2), :] + 0.5 * val).astype(BF16)
            cp_out(t, c).start()

    @pl.loop(0, NT)
    def _(t):
        cp_out(t, 0).wait()
        cp_out(t, 1).wait()


@jax.jit
def pallas_sequential_preLN__sliding_local_dilated__glu_gated_geglu__prompt_kernel(
        A_x, A_wqkv, A_wo, B_x, B_w_gate, B_w_up, B_w_down):
    del B_x
    any_spec = pl.BlockSpec(memory_space=pl.ANY)
    out = pl.pallas_call(
        _kernel,
        in_specs=[any_spec] * 6,
        out_specs=any_spec,
        out_shape=jax.ShapeDtypeStruct((S, D), A_x.dtype),
        scratch_shapes=[
            pltpu.VMEM((S, D), BF16),
            pltpu.VMEM((3 * D, D), BF16),
            pltpu.VMEM((7, D // 4, D // 2), U32),
            pltpu.VMEM((7, D // 2, D // 2), U32),
            pltpu.VMEM((7, D // 4, D // 2), U32),
            pltpu.VMEM((D, F), BF16),
            pltpu.VMEM((D, F), BF16),
            pltpu.VMEM((F, D + 128), BF16),
            pltpu.VMEM((H * PITCH_C + 32, 128), U32),
            pltpu.VMEM((2, H * PITCH_R + 32, 128), U32),
            pltpu.VMEM((26 * NJ // 4, (S + T) // 4, 128), U32),
            pltpu.VMEM((2 * NJ, P0 + S, 128), F32),
            pltpu.VMEM((NJ, P0 + S, 128), F32),
            pltpu.VMEM((W, T, 128), F32),
            pltpu.VMEM((T + S, D), F32),
            pltpu.VMEM((NJ, T + S, 128), F32),
            pltpu.VMEM((26, T // 4, F // 4), U32),
            pltpu.SemaphoreType.DMA((NT,)),
            pltpu.SemaphoreType.DMA((3 * NS,)),
            pltpu.SemaphoreType.DMA(()),
            pltpu.SemaphoreType.DMA((3,)),
            pltpu.SemaphoreType.DMA((2 * NT,)),
        ],
        compiler_params=pltpu.CompilerParams(vmem_limit_bytes=120 * 1024 * 1024),
    )(A_x.reshape(S, D), A_wqkv, A_wo, B_w_gate, B_w_up, B_w_down)
    return out.reshape(A_x.shape)
```
